```python
import jax
import jax.numpy as jnp

def _softmax(x, axis=-1):
    return jax.nn.softmax(x, axis=axis)
def _gelu(x):
    return jax.nn.gelu(x, approximate=True)
def _silu(x):
    return jax.nn.silu(x)
def _sigmoid(x):
    return jax.nn.sigmoid(x)
def _layernorm(x, axis=-1, eps=1e-5):
    m = jnp.mean(x, axis=axis, keepdims=True)
    v = jnp.var(x, axis=axis, keepdims=True)
    return (x - m) / jnp.sqrt(v + eps)
def _scatter_add(tgt, idx, src, axis=0):
    return tgt.at[idx].add(src)
def _segment_sum(src, seg, n):
    return jax.ops.segment_sum(src, seg, n)
class _Rng:
    def __init__(self, key):
        self._k = key
    def _next(self):
        self._k, sub = jax.random.split(self._k)
        return sub
    def normal(self, shape):
        return jax.random.normal(self._next(), shape, dtype=jnp.bfloat16)
    def randint(self, lo, hi, shape):
        return jax.random.randint(self._next(), shape, lo, hi, dtype=jnp.int32)
    def uniform(self, shape, lo=0.0, hi=1.0):
        return jax.random.uniform(self._next(), shape, jnp.bfloat16, lo, hi)
    def permutation(self, n):
        return jax.random.permutation(self._next(), n)


kernel_name = 'parallel_sum__compressed_kv_cla__moe_arch_mod__prompt'

def _fwd_setup_inputs():
    _rng = _Rng(jax.random.key(int.from_bytes(__import__("os").urandom(4), "little")))
    _w = (lambda a: (lambda t: t.astype(jnp.bfloat16) if jnp.issubdtype(t.dtype, jnp.floating) else t)(jnp.asarray(a)))
    def _A_setup():
        B, H, Sq, Sk, D, M = 1, 32, 2048, 2048, 128, 576
        Dc = 4 * D
        return {
            "x": _w((lambda *s: _rng.normal(s) * 0.05)(B, Sq, M)),
            "c_kv": _w((lambda *s: _rng.normal(s) * 0.05)(B, Sk, Dc)),
            "w_q": _w((lambda *s: _rng.normal(s) * 0.05)(M, H, D) * (M ** -0.5)),
            "w_uk": _w((lambda *s: _rng.normal(s) * 0.05)(Dc, H, D) * (Dc ** -0.5)),
            "w_uv": _w((lambda *s: _rng.normal(s) * 0.05)(Dc, H, D) * (Dc ** -0.5)),
            "w_o": _w((lambda *s: _rng.normal(s) * 0.05)(H, D, M) * ((H * D) ** -0.5)),
        }
    _A_in = _A_setup()

    def _B_setup():
        B, S, D, F, C = 1, 2048, 576, 4608, 8
        return {
            "x": _w((lambda *s: _rng.normal(s) * 0.05)(B, S, D)),
            "w_r": _w((lambda *s: _rng.normal(s) * 0.05)(D)),
            "w_gate": _w((lambda *s: _rng.normal(s) * 0.05)(D, F)),
            "w_up": _w((lambda *s: _rng.normal(s) * 0.05)(D, F)),
            "w_down": _w((lambda *s: _rng.normal(s) * 0.05)(F, D)),
        }
    _B_in = _B_setup()

    return {
        "A_x": _A_in["x"],
        "A_c_kv": _A_in["c_kv"],
        "A_w_q": _A_in["w_q"],
        "A_w_uk": _A_in["w_uk"],
        "A_w_uv": _A_in["w_uv"],
        "A_w_o": _A_in["w_o"],
        "B_x": _B_in["x"],
        "B_w_r": _B_in["w_r"],
        "B_w_gate": _B_in["w_gate"],
        "B_w_up": _B_in["w_up"],
        "B_w_down": _B_in["w_down"],
    }

def _fwd_reference(A_x, A_c_kv, A_w_q, A_w_uk, A_w_uv, A_w_o, B_x, B_w_r, B_w_gate, B_w_up, B_w_down):
    def _A_ref(x, c_kv, w_q, w_uk, w_uv, w_o):
        B, Sq, M = x.shape[0], x.shape[1], x.shape[2]
        Sk = c_kv.shape[1]
        H, D = w_q.shape[1], w_q.shape[2]
        q = jnp.einsum("bqm,mhd->bhqd", x, w_q)
        k = jnp.einsum("bkc,chd->bhkd", c_kv, w_uk)
        v = jnp.einsum("bkc,chd->bhkd", c_kv, w_uv)
        scores = jnp.einsum("bhqd,bhkd->bhqk", q, k) * (D ** -0.5)
        off = Sk - Sq
        qi = jnp.arange(Sq)[:, None]
        kj = jnp.arange(Sk)[None, :]
        cmask = kj <= (qi + off)
        scores = jnp.where(cmask[None, None], scores, -1e9)
        p = _softmax(scores, axis=-1)
        ctx = jnp.einsum("bhqk,bhkd->bhqd", p, v)
        return jnp.einsum("bhqd,hdm->bqm", ctx, w_o)

    def _B_ref(x, w_r, w_gate, w_up, w_down):
        B, S, D = x.shape
        C = 8
        r = x @ w_r
        idx = jnp.argsort(jax.lax.stop_gradient(-r), axis=-1)[:, :C]
        idx_e = jnp.repeat(idx.reshape(B, C, 1), D, axis=2)
        x_sel = jnp.take_along_axis(x, idx_e, axis=1)
        g = _silu(x_sel @ w_gate)
        u = x_sel @ w_up
        y = (g * u) @ w_down
        r_sel = _sigmoid(jnp.take_along_axis(r, idx, axis=1))
        y = y * r_sel.reshape(B, C, 1)
        b_off = (jnp.arange(B) * S).reshape(B, 1)
        flat_idx = (idx + b_off).reshape(B * C)
        zero = (x * 0.0).reshape(B * S, D)
        upd = _scatter_add(zero, flat_idx, y.reshape(B * C, D), axis=0)
        return x + upd.reshape(B, S, D)

    x = A_x
    xn = _layernorm(x, axis=-1)
    return x + _A_ref(xn, A_c_kv, A_w_q, A_w_uk, A_w_uv, A_w_o) + _B_ref(xn, B_w_r, B_w_gate, B_w_up, B_w_down)


def setup_inputs():
    _inp = _fwd_setup_inputs()
    _gk = jax.random.fold_in(jax.random.key(int.from_bytes(__import__("os").urandom(4), "little")), 2**31 - 1)
    _shapes = [[1, 2048, 576]]
    _dtypes = ['bfloat16']
    _gks = jax.random.split(_gk, len(_shapes))
    _gs = [jax.random.normal(k, s, dtype=jnp.dtype(d)) * 0.05 for k, s, d in zip(_gks, _shapes, _dtypes)]
    _inp["grad_out"] = _gs[0]
    return _inp

def reference(A_x, A_c_kv, A_w_q, A_w_uk, A_w_uv, A_w_o, B_w_r, B_w_gate, B_w_up, B_w_down, B_x, grad_out):
    _const = dict(B_x=B_x)
    def _f(*_d):
        return _fwd_reference(**{'A_x': _d[0], 'A_c_kv': _d[1], 'A_w_q': _d[2], 'A_w_uk': _d[3], 'A_w_uv': _d[4], 'A_w_o': _d[5], 'B_w_r': _d[6], 'B_w_gate': _d[7], 'B_w_up': _d[8], 'B_w_down': _d[9], **_const})
    _out, _vjp = jax.vjp(_f, A_x, A_c_kv, A_w_q, A_w_uk, A_w_uv, A_w_o, B_w_r, B_w_gate, B_w_up, B_w_down)
    _grads = _vjp(grad_out)
    _out0 = jnp.asarray(_out)
    return (_out0, *[jnp.asarray(_g) for _g in _grads])
```

```python
import functools, math
import jax, jax.numpy as jnp
from jax import lax
import jax.experimental.pallas as pl
import jax.experimental.pallas.tpu as pltpu

S, M, H, D, DC, F, C = 2048, 576, 32, 128, 512, 4608, 8
T = 128
NB = S // T
FC = 256
NFC = F // FC
CP = 16
G = 8
NG = H // G
f32, bf16, u32, i32 = jnp.float32, jnp.bfloat16, jnp.uint32, jnp.int32
LOG2E = math.log2(math.e)
LN2 = math.log(2.0)
SCALE = D ** -0.5
QSCALE = SCALE * LOG2E
EPS_B = 1.0013580322265625e-05
WROWS = (M, DC, DC)
V = pltpu.VMEM

def nn(a, b): return lax.dot_general(a, b, (((1,), (0,)), ((), ())), preferred_element_type=f32)
def nt(a, b): return lax.dot_general(a, b, (((1,), (1,)), ((), ())), preferred_element_type=f32)
def rb(x): return x.astype(bf16).astype(f32)
def sigmoid(x): return 1.0 / (1.0 + jnp.exp(-x))

class Pk:
    def __init__(self, ref):
        self.ref = ref
        self.shape = (ref.shape[0] * 2, ref.shape[1])
    def _ix(self, idx):
        if idx is Ellipsis:
            return (slice(None), slice(None))
        r, c = idx
        if isinstance(r, tuple):
            return (pl.ds(pl.multiple_of(r[0] * (r[1] // 2), 8), r[1] // 2), c)
        r0 = 0 if r.start is None else r.start
        r1 = self.shape[0] if r.stop is None else r.stop
        assert r0 % 16 == 0 and r1 % 16 == 0
        return (slice(r0 // 2, r1 // 2), c)
    def __getitem__(self, idx):
        return pltpu.bitcast(self.ref[self._ix(idx)], bf16)
    def __setitem__(self, idx, val):
        self.ref[self._ix(idx)] = pltpu.bitcast(val.astype(bf16), u32)

def PkV(r, c): return pltpu.VMEM((r // 2, c), u32)

SCR = dict(
    st_x=V((M, S), bf16), st_go=V((M, S), bf16), st_c=V((S, DC), bf16),
    wi0=V((M, G, D), bf16), wi1=V((DC, G, D), bf16), wi2=V((DC, G, D), bf16),
    wo0=V((M, G, D), bf16), wo1=V((DC, G, D), bf16), wo2=V((DC, G, D), bf16),
    wf0=V((2 * M * 4, D), u32), wf1=V((2 * DC * 4, D), u32), wf2=V((2 * DC * 4, D), u32),
    df0=V((2 * M * 4, D), u32), df1=V((2 * DC * 4, D), u32), df2=V((2 * DC * 4, D), u32),
    woi=V((2, M, D), bf16), woo=V((2, M, D), bf16),
    mi=V((2, 3, M, FC), bf16), mo=V((2, 3, M, FC), bf16),
    xnT=PkV(M, S), goT=PkV(M, S), c=PkV(S, DC), cT=PkV(DC, S), rstd=V((1, S), f32),
    outT=V((M, S), f32), dxnT=V((M, S), f32), dc=V((S, DC), f32),
    oh=V((CP, S), bf16), xsel=V((CP, M), bf16), xselT=V((M, CP), bf16), gosel=V((CP, M), f32),
    dy=V((CP, M), bf16), dyT=V((M, CP), bf16), rs=V((CP, 128), f32), y=V((CP, M), f32), dxsel=V((CP, M), f32),
    wqT=PkV(D, 640), wo=PkV(D, 640), wq=PkV(M, D), woT=PkV(M, D), wkv=PkV(DC, 2 * D),
    qT=PkV(D, S), dctxT=V((D, S), f32), k=PkV(S, D), v=PkV(S, D), kT=PkV(D, S), vT=PkV(D, S),
    sT0=V((S, 512), f32), sT1=V((S, 512), f32), PT=PkV(S, S), dST=PkV(S, S),
    ctxT=PkV(D, S), dqT=PkV(D, S), dcs=PkV(D, S), dkv=PkV(S, 2 * D),
    dwq=V((M, D), f32), dwo=V((M, D), f32), dwkv=V((DC, 2 * D), f32),
    sem=pltpu.SemaphoreType.DMA((32,)),
)
PACKED = ("xnT", "goT", "c", "cT", "wqT", "wo", "wq", "woT", "wkv", "qT", "k", "v", "kT", "vT", "PT", "dST",
          "ctxT", "dqT", "dcs", "dkv")
PIN = ("wqT", "wo", "wq", "woT", "wkv", "qT", "dctxT", "k", "v", "kT", "vT", "sT0", "sT1", "PT", "dST",
       "ctxT", "dqT", "dcs", "dkv", "dwq", "dwo", "dwkv")

ORD4 = ("K0 K1 K2 K3 Q3 O3 A3 V0 V1 V2 V3 Q2 O2 X3 A2 B3 Q1 O1 X2 A1 B2 Q0 O0 X1 C3 A0 B1 D3 X0 EV3 C2 B0 OUT3 DWO3 D2 EK3 C1 "
        "DXN3 DWQ3 EV2 D1 C0 OUT2 DWO2 EK2 DXN2 DWQ2 D0 EV1 EK1 DCK3 DWK3 EV0 EK0 OUT1 DWO1 DXN1 DWQ1 DCK2 DWK2 OUT0 DWO0 DXN0 DWQ0 DCK1 DWK1 DCK0 DWK0")


class NS:
    def __init__(self, d):
        self._d = d
    def __getattr__(self, n):
        return self._d[n]


def make(cfg):
    names = list(SCR)

    def kernel(xT_h, c_h, goT_h, wq_h, wuk_h, wuv_h, woT_h, wr_ref, wg_h, wu_h, wdT_h,
               outT_h, dxT_h, dc_h, dwq_h, dwuk_h, dwuv_h, dwoT_h, dwr_ref, dwg_h, dwu_h, dwdT_h, *scr):
        raw = dict(zip(names, scr))
        s = NS({n: Pk(raw[n]) if n in PACKED else raw[n] for n in names})
        al = slice(None)
        sem = s.sem
        w_h = (wq_h, wuk_h, wuv_h); dw_h = (dwq_h, dwuk_h, dwuv_h)
        wi = (s.wi0, s.wi1, s.wi2); wo = (s.wo0, s.wo1, s.wo2)
        wf = (s.wf0, s.wf1, s.wf2); df = (s.df0, s.df1, s.df2)
        m_h = (wg_h, wu_h, wdT_h); dm_h = (dwg_h, dwu_h, dwdT_h)
        cp = pltpu.make_async_copy
        XW = 512; NX = S // XW

        def x_in(b): return cp(xT_h.at[:, pl.ds(pl.multiple_of(b * XW, XW), XW)], s.st_x.at[:, pl.ds(pl.multiple_of(b * XW, XW), XW)], sem.at[16 + b])
        def go_in(b): return cp(goT_h.at[:, pl.ds(pl.multiple_of(b * XW, XW), XW)], s.st_go.at[:, pl.ds(pl.multiple_of(b * XW, XW), XW)], sem.at[20 + b])
        def c_in(b): return cp(c_h.at[pl.ds(pl.multiple_of(b * XW, XW), XW), :], s.st_c.at[pl.ds(pl.multiple_of(b * XW, XW), XW), :], sem.at[24 + b])
        def w_in_full(w): return cp(w_h[w].at[:, pl.ds(0, G), :], wi[w], sem.at[w])
        def w_in(w, t):
            n = WROWS[w] // G
            g = jnp.minimum((t >> 3) + 1, NG - 1)
            r = pl.ds((t & 7) * n, n)
            return cp(w_h[w].at[r, pl.ds(pl.multiple_of(g * G, G), G), :], wi[w].at[r], sem.at[w])
        def w_out(w, t):
            n = WROWS[w] // G
            g = jnp.maximum((t >> 3) - 1, 0)
            r = pl.ds((t & 7) * n, n)
            return cp(wo[w].at[r], dw_h[w].at[r, pl.ds(pl.multiple_of(g * G, G), G), :], sem.at[3 + w])
        def w_out_full(w): return cp(wo[w], dw_h[w].at[:, pl.ds((NG - 1) * G, G), :], sem.at[3 + w])
        def wo_in(t): return cp(woT_h.at[jnp.minimum(t, H - 1)], s.woi.at[t & 1], sem.at[6])
        def wo_out(t): return cp(s.woo.at[t & 1], dwoT_h.at[t], sem.at[7])
        def m_in(w, t): return cp(m_h[w].at[:, pl.ds(pl.multiple_of(t * FC, FC), FC)], s.mi.at[t & 1, w], sem.at[8 + w])
        def m_out(w, t): return cp(s.mo.at[t & 1, w], dm_h[w].at[:, pl.ds(pl.multiple_of(t * FC, FC), FC)], sem.at[11 + w])

        def cvt_in(w, slot, sl_):
            n = WROWS[w] // G
            x = wi[w][pl.ds(sl_ * n, n)].reshape(n * G, D)
            wf[w][pl.ds(pl.multiple_of(slot * (WROWS[w] * 4) + sl_ * (n * 4), 8), n * 4), :] = pltpu.bitcast(x, u32)
        def cvt_out(w, slot, sl_):
            n = WROWS[w] // G
            x = df[w][pl.ds(pl.multiple_of(slot * (WROWS[w] * 4) + sl_ * (n * 4), 8), n * 4), :]
            wo[w][pl.ds(sl_ * n, n)] = pltpu.bitcast(x, bf16).reshape(n, G, D)

        for b in range(NX): x_in(b).start()
        for b in range(NX): go_in(b).start()
        for b in range(NX): c_in(b).start()
        for w in range(3): w_in_full(w).start()
        wo_in(0).start()
        for w in range(3): m_in(w, 0).start()

        @pl.loop(0, NX)
        def _(bb):
            x_in(bb).wait()
            @pl.loop(0, XW // T)
            def _(b4):
                b = bb * (XW // T) + b4
                cs = pl.ds(pl.multiple_of(b * T, T), T)
                x = s.st_x[:, cs].astype(f32)
                mu = jnp.mean(x, axis=0, keepdims=True)
                xc32 = x - mu
                var = jnp.mean(xc32 * xc32, axis=0, keepdims=True)
                sd = rb(jnp.sqrt(rb(rb(var) + EPS_B)))
                xn = (rb(x - rb(mu)) / sd).astype(bf16)
                s.xnT[al, cs] = xn
                s.rstd[:, cs] = 1.0 / sd
                s.outT[:, cs] = x + xn.astype(f32)
                for n in PIN:
                    raw[n][pl.ds(pl.multiple_of((b & 1) * 8, 8), 8), 0:128] = jnp.zeros((8, 128), raw[n].dtype)

        wr = jnp.broadcast_to(wr_ref[...], (CP, M))
        r = rb(nn(wr, s.xnT[...])[0:1, :])
        r = jnp.concatenate([r[:, i * 256:(i + 1) * 256] for i in range(8)], axis=0)
        col = (lax.broadcasted_iota(i32, (8, 256), 0) * 256 + lax.broadcasted_iota(i32, (8, 256), 1)).astype(f32)
        colf = lax.broadcasted_iota(i32, (CP, S), 1).astype(f32)
        row = lax.broadcasted_iota(i32, (CP, 1), 0)
        idxs = jnp.full((CP, 1), -1.0, f32)
        rsel = jnp.zeros((CP, 1), f32)
        for t in range(C):
            mx = jnp.max(jnp.max(r, axis=0, keepdims=True), axis=1, keepdims=True)
            ix = jnp.min(jnp.min(jnp.where(r == mx, col, float(S)), axis=0, keepdims=True), axis=1, keepdims=True)
            r = jnp.where(col == ix, -jnp.inf, r)
            idxs = jnp.where(row == t, ix, idxs)
            rsel = jnp.where(row == t, mx, rsel)
        oh = jnp.where(colf == idxs, 1.0, 0.0).astype(bf16)
        s.oh[...] = oh
        rs = sigmoid(rsel)
        s.rs[...] = jnp.broadcast_to(rs, s.rs.shape)

        @pl.loop(0, NX)
        def _(bb):
            go_in(bb).wait()
            @pl.loop(0, XW // T)
            def _(b4):
                cs = pl.ds(pl.multiple_of((bb * (XW // T) + b4) * T, T), T)
                go = s.st_go[:, cs]
                s.goT[al, cs] = go
                s.dxnT[:, cs] = go.astype(f32)

        xsel = nt(s.oh[...], s.xnT[...])
        s.xsel[...] = xsel.astype(bf16)
        gosel = nt(s.oh[...], s.goT[...])
        s.gosel[...] = gosel
        dy = gosel * s.rs[:, 0:1]
        s.dy[...] = dy.astype(bf16)
        s.xselT[...] = xsel.T.astype(bf16)
        s.dyT[...] = dy.T.astype(bf16)
        s.y[...] = jnp.zeros_like(s.y)
        s.dxsel[...] = jnp.zeros_like(s.dxsel)

        @pl.loop(0, NX)
        def _(bb):
            c_in(bb).wait()
            @pl.loop(0, XW // T)
            def _(b4):
                b = bb * (XW // T) + b4
                cs = pl.ds(pl.multiple_of(b * T, T), T)
                cb = s.st_c[cs, :]
                s.c[(b, T), al] = cb
                s.cT[al, cs] = cb.T
                s.dc[cs, :] = jnp.zeros((T, DC), f32)

        for w in range(3): w_in_full(w).wait()
        for w in range(3): cvt_in(w, 0, 0)
        for w in range(3): w_in(w, 0).start()
        @pl.loop(1, G)
        def _(i):
            for w in range(3): cvt_in(w, 0, i)

        @pl.loop(0, H)
        def _(h):
            g = h >> 3
            for w in range(3): w_in(w, h).wait()
            wo_in(h).wait()
            @pl.when(h >= G + 2)
            def _():
                for w in range(3): w_out(w, h - 2).wait()
            @pl.when(h >= 2)
            def _():
                wo_out(h - 2).wait()
            for w in range(3): w_in(w, h + 1).start()
            wo_in(h + 1).start()
            @pl.when(h >= G + 1)
            def _():
                for w in range(3): w_out(w, h - 1).start()
            @pl.when(h >= 1)
            def _():
                wo_out(h - 1).start()

            @pl.when(h < NFC)
            def _moe():
                for w in range(3): m_in(w, h).wait()
                @pl.when(h + 1 < NFC)
                def _():
                    for w in range(3): m_in(w, h + 1).start()
                @pl.when(h >= 1)
                def _():
                    for w in range(3): m_out(w, h - 1).wait()
                sl_ = h & 1
                wg = s.mi[sl_, 0]; wu = s.mi[sl_, 1]; wdT = s.mi[sl_, 2]
                xs = s.xsel[...]
                a = nn(xs, wg); u = nn(xs, wu)
                dh = nn(s.dy[...], wdT)
                sg = sigmoid(a)
                g_ = a * sg
                hb = (g_ * u).astype(bf16)
                da = (dh * u * (sg * (1.0 + a * (1.0 - sg)))).astype(bf16)
                du = (dh * g_).astype(bf16)
                s.y[...] += nt(hb, wdT)
                s.dxsel[...] += nt(da, wg) + nt(du, wu)
                s.mo[sl_, 0] = nn(s.xselT[...], da).astype(bf16)
                s.mo[sl_, 1] = nn(s.xselT[...], du).astype(bf16)
                s.mo[sl_, 2] = nn(s.dyT[...], hb).astype(bf16)
                for w in range(3): m_out(w, h).start()

            odd = h & 1
            sh = (16 * (1 - odd)).astype(u32)
            pr = (h & 7) >> 1
            def w_load(w):
                x = wf[w][pl.ds((g & 1) * (WROWS[w] * 4) + pr, WROWS[w], stride=4), :]
                return pltpu.bitcast((x << sh) & jnp.uint32(0xFFFF0000), f32).astype(bf16)
            def w_store(w, val):
                ix = pl.ds((g & 1) * (WROWS[w] * 4) + pr, WROWS[w], stride=4)
                bits = pltpu.bitcast(rb(val), u32) >> sh
                df[w][ix, :] = jnp.where(odd == 1, df[w][ix, :], jnp.uint32(0)) | bits
            def side():
                for w in range(3): cvt_in(w, (g + 1) & 1, h & 7)
                for w in range(3): cvt_out(w, (g + 1) & 1, h & 7)
            head_body(cfg, s, h, w_load, w_store, side)

        for w in range(3): w_in(w, H).wait()
        wo_in(H).wait()
        for w in range(3): w_out(w, H - 2).wait()
        wo_out(H - 2).wait()
        for w in range(3): w_out(w, H - 1).start()
        wo_out(H - 1).start()
        for w in range(3): m_out(w, NFC - 1).wait()

        def o_x(b): return cp(s.st_x.at[:, pl.ds(pl.multiple_of(b * XW, XW), XW)], outT_h.at[:, pl.ds(pl.multiple_of(b * XW, XW), XW)], sem.at[16 + b])
        def o_go(b): return cp(s.st_go.at[:, pl.ds(pl.multiple_of(b * XW, XW), XW)], dxT_h.at[:, pl.ds(pl.multiple_of(b * XW, XW), XW)], sem.at[20 + b])
        def o_c(b): return cp(s.st_c.at[pl.ds(pl.multiple_of(b * XW, XW), XW), :], dc_h.at[pl.ds(pl.multiple_of(b * XW, XW), XW), :], sem.at[24 + b])

        @pl.loop(0, NX)
        def _(bb):
            @pl.loop(0, XW // T)
            def _(b4):
                cs = pl.ds(pl.multiple_of((bb * (XW // T) + b4) * T, T), T)
                s.st_c[cs, :] = s.dc[cs, :].astype(bf16)
            o_c(bb).start()
        for w in range(3): w_out(w, H - 1).wait()
        @pl.loop(0, G)
        def _(i):
            for w in range(3): cvt_out(w, (NG - 1) % 2, i)
        for w in range(3): w_out_full(w).start()

        rs = s.rs[:, 0:1]
        y = s.y[...]
        drs = jnp.sum(s.gosel[...] * y, axis=1, keepdims=True)
        dr = drs * rs * (1.0 - rs)
        wr = wr_ref[...].astype(f32)
        dwr_ref[...] = jnp.sum(dr * s.xsel[...].astype(f32), axis=0, keepdims=True).astype(bf16)
        s.xselT[...] = (y * rs).T.astype(bf16)
        s.dyT[...] = (s.dxsel[...] + dr * wr).T.astype(bf16)

        @pl.loop(0, NX)
        def _(bb):
            @pl.loop(0, XW // T)
            def _(b4):
                cs = pl.ds(pl.multiple_of((bb * (XW // T) + b4) * T, T), T)
                oh = s.oh[:, cs]
                s.st_x[:, cs] = (s.outT[:, cs] + nn(s.xselT[...], oh)).astype(bf16)
                xn = s.xnT[al, cs].astype(f32)
                dxn = s.dxnT[:, cs] + nn(s.dyT[...], oh)
                m1 = jnp.mean(dxn, axis=0, keepdims=True)
                m2 = jnp.mean(dxn * xn, axis=0, keepdims=True)
                go = s.goT[al, cs].astype(f32)
                s.st_go[:, cs] = (go + s.rstd[:, cs] * (dxn - m1 - xn * m2)).astype(bf16)
            o_x(bb).start()
            o_go(bb).start()
        for b in range(NX):
            o_c(b).wait(); o_x(b).wait(); o_go(b).wait()
        for w in range(3): w_out_full(w).wait()
        wo_out(H - 1).wait()

    def fn(A_x, A_c_kv, A_w_q, A_w_uk, A_w_uv, A_w_o, B_x, B_w_r, B_w_gate, B_w_up, B_w_down, grad_out):
        xT = A_x.reshape(S, M).T; goT = grad_out.reshape(S, M).T; c = A_c_kv.reshape(S, DC)
        woT = jnp.swapaxes(A_w_o, 1, 2)
        wr = B_w_r.reshape(1, M)
        wdT = B_w_down.T
        sds = jax.ShapeDtypeStruct
        hbm = pl.BlockSpec(memory_space=pl.ANY)
        vm = pl.BlockSpec(memory_space=pltpu.VMEM)
        outs = pl.pallas_call(
            kernel,
            in_specs=[hbm] * 7 + [vm] + [hbm] * 3,
            out_specs=[hbm] * 7 + [vm] + [hbm] * 3,
            out_shape=[sds((M, S), bf16), sds((M, S), bf16), sds((S, DC), bf16), sds((M, H, D), bf16),
                       sds((DC, H, D), bf16), sds((DC, H, D), bf16), sds((H, M, D), bf16), sds((1, M), bf16),
                       sds((M, F), bf16), sds((M, F), bf16), sds((M, F), bf16)],
            scratch_shapes=list(SCR.values()),
            compiler_params=pltpu.CompilerParams(vmem_limit_bytes=120 * 1024 * 1024),
            name="mla",
        )(xT, c, goT, A_w_q, A_w_uk, A_w_uv, woT, wr, B_w_gate, B_w_up, wdT)
        outT, dxT, dc, dwq, dwuk, dwuv, dwoT, dwr, dwg, dwu, dwdT = outs
        return (outT.T.reshape(1, S, M), dxT.T.reshape(1, S, M), dc.reshape(1, S, DC), dwq, dwuk, dwuv,
                jnp.swapaxes(dwoT, 1, 2), dwr.reshape(M), dwg, dwu, dwdT.T)
    return fn


def head_body(cfg, s, h, w_load, w_store, side):
    al = slice(None)
    sl = lambda a, b: slice(a * T, b * T)
    tri = lax.broadcasted_iota(i32, (T, T), 0) <= lax.broadcasted_iota(i32, (T, T), 1)
    never = lax.broadcasted_iota(i32, (8, T), 0) + h < 0
    st = {}
    order = cfg.get("order", ORD4)
    seen = set()
    GE = cfg.get("G", 16)
    toks = []
    sT = (s.sT0, s.sT1)

    def tree(op, xs):
        xs = list(xs)
        while len(xs) > 1:
            xs = [op(xs[i], xs[i + 1]) if i + 1 < len(xs) else xs[i] for i in range(0, len(xs), 2)]
        return xs[0]
    def vregs(x):
        return [x[8 * i:8 * i + 8, :] for i in range(x.shape[0] // 8)]
    def tok(x, colmajor=True):
        nc = x.shape[1] // T if colmajor else 1
        for c in range(nc):
            for i in range(x.shape[0] // 8):
                toks.append((x, i, c))
        return x
    def get_tok(t):
        x, i, c = t
        return x[8 * i:8 * i + 8, c * T:(c + 1) * T]

    def W():
        s.wkv[al, :D] = w_load(1); s.wkv[al, D:] = w_load(2)
        wq = w_load(0); woT = s.woi[h & 1]
        s.wq[...] = wq; s.woT[...] = woT
        s.wqT[al, :M] = s.wq[...].T; s.wo[al, :M] = s.woT[...].T
    def K(J):
        r = sl(4 * J, 4 * J + 4)
        s.k[r, al] = tok(nn(s.c[r, al], s.wkv[al, :D]))
        s.kT[al, r] = s.k[r, al].T
    def Vv(J):
        r = sl(4 * J, 4 * J + 4)
        s.v[r, al] = tok(nn(s.c[r, al], s.wkv[al, D:]))
        s.vT[al, r] = s.v[r, al].T
    def Q(J):
        r = sl(4 * J, 4 * J + 4)
        s.qT[al, r] = tok(nn(s.wqT[al, :M], s.xnT[al, r])) * QSCALE
    def O(J):
        r = sl(4 * J, 4 * J + 4)
        s.dctxT[:, r] = tok(nn(s.wo[al, :M], s.goT[al, r]))
    def A(J):
        for j in range(4 * J + 3, 4 * J - 1, -1):
            x = nn(s.k[sl(0, j + 1), al], s.qT[al, sl(j, j + 1)])
            if j == 4 * J + 3: tok(x)
            sd = jnp.where(tri, x[j * T:, :], -1e9)
            x = sd if j == 0 else jnp.concatenate([x[:j * T, :], sd], axis=0)
            vs = vregs(x); a = vs[0]
            for y in vs[1:]:
                a = jnp.maximum(a, y)
            st["m", j] = jnp.broadcast_to(jnp.max(a, axis=0, keepdims=True), (8, T))
            sT[J % 2][sl(0, j + 1), sl(j - 4 * J, j - 4 * J + 1)] = x
        st["tok0", J] = len(toks)
    def X(J):
        tk = toks[st["tok0", J] + cfg.get("skip", 8): len(toks) - cfg.get("tail", 32)]
        ng = sum(16 * (j + 1) // GE for j in range(4 * J, 4 * J + 4))
        g = 0
        for j in range(4 * J + 3, 4 * J - 1, -1):
            cs = sl(j, j + 1)
            l = None; m = st["m", j]
            for t in range(j + 1):
                sv = vregs(sT[J % 2][sl(t, t + 1), sl(j - 4 * J, j - 4 * J + 1)])
                ps = []
                for i in range(0, 16, GE):
                    m = jnp.where(never, get_tok(tk[g * len(tk) // ng]), m); g += 1
                    grp = [jnp.exp2(x - m) for x in sv[i:i + GE]]
                    s_ = tree(jnp.add, grp)
                    l = s_ if l is None else l + s_
                    ps += grp
                s.PT[sl(t, t + 1), cs] = jnp.concatenate(ps, axis=0)
            inv_l = 1.0 / jnp.sum(l, axis=0, keepdims=True)
            st["il", j] = inv_l
            s.dcs[al, cs] = s.dctxT[:, cs] * inv_l
    def B(J):
        for j in range(4 * J + 3, 4 * J - 1, -1):
            cs = sl(j, j + 1)
            a = None
            for t0 in range(0, j + 1, 4):
                t1 = min(t0 + 4, j + 1)
                x = tok(nn(s.vT[al, sl(t0, t1)], s.PT[sl(t0, t1), cs]))
                a = x if a is None else a + x
            ctxT = a * st["il", j]
            st["dl", j] = jnp.sum(ctxT * s.dcs[al, cs].astype(f32), axis=0, keepdims=True)
            s.ctxT[al, cs] = ctxT
    def Cc(J):
        for j in range(4 * J + 3, 4 * J - 1, -1):
            cs = sl(j, j + 1); r = sl(0, j + 1)
            dpT = nn(s.v[r, al], s.dcs[al, cs])
            if j == 4 * J + 3: tok(dpT)
            s.dST[r, cs] = s.PT[r, cs].astype(f32) * (dpT - st["dl", j])
    def Dd(J):
        for j in range(4 * J + 3, 4 * J - 1, -1):
            cs = sl(j, j + 1)
            a = None
            for t0 in range(0, j + 1, 4):
                t1 = min(t0 + 4, j + 1)
                x = tok(nn(s.kT[al, sl(t0, t1)], s.dST[sl(t0, t1), cs]))
                a = x if a is None else a + x
            s.dqT[al, cs] = a * SCALE
    def EV(I):
        for i in range(4 * I + 3, 4 * I - 1, -1):
            s.dkv[sl(i, i + 1), D:] = tok(nt(s.PT[sl(i, i + 1), sl(i, NB)], s.dcs[al, sl(i, NB)]))
    def EK(I):
        for i in range(4 * I + 3, 4 * I - 1, -1):
            s.dkv[sl(i, i + 1), :D] = tok(nt(s.dST[sl(i, i + 1), sl(i, NB)], s.qT[al, sl(i, NB)])) * LN2
    def acc(name, a_ref, o_fn, val):
        cnt = sum(1 for x in seen if x[0] == name)
        if cnt == 0: a_ref[...] = val
        elif cnt < 3: a_ref[...] += val
        else: o_fn(a_ref[...] + val)
    def OUT(J):
        r = sl(4 * J, 4 * J + 4)
        s.outT[:, r] += tok(nn(s.woT[...], s.ctxT[al, r]), False)
    def DWO(J):
        r = sl(4 * J, 4 * J + 4)
        def fin(x): s.woo[h & 1] = x.astype(bf16)
        acc("DWO", s.dwo, fin, tok(nt(s.goT[al, r], s.ctxT[al, r])))
    def DXN(J):
        r = sl(4 * J, 4 * J + 4)
        s.dxnT[:, r] += tok(nn(s.wq[...], s.dqT[al, r]), False)
    def DWQ(J):
        r = sl(4 * J, 4 * J + 4)
        acc("DWQ", s.dwq, lambda x: w_store(0, x), tok(nt(s.xnT[al, r], s.dqT[al, r])))
    def DCK(I):
        r = sl(4 * I, 4 * I + 4)
        s.dc[r, :] += nt(s.dkv[r, al], s.wkv[...])
    def DWK(I):
        r = sl(4 * I, 4 * I + 4)
        def fin(x):
            w_store(1, x[:, :D]); w_store(2, x[:, D:])
        acc("DWK", s.dwkv, fin, nn(s.cT[al, r], s.dkv[r, al]))
    ops = dict(K=K, V=Vv, Q=Q, O=O, A=A, X=X, B=B, C=Cc, D=Dd, EV=EV, EK=EK, OUT=OUT, DWO=DWO, DXN=DXN, DWQ=DWQ, DCK=DCK, DWK=DWK)
    W()
    side()
    for tk_ in order.split():
        name, J = tk_[:-1], int(tk_[-1])
        assert (name, J) not in seen
        ops[name](J)
        seen.add((name, J))
    assert len(seen) == 4 * len(ops), len(seen)


_impl = make(dict())


@jax.jit
def pallas_parallel_sum__compressed_kv_cla__moe_arch_mod__prompt_kernel(
        A_x, A_c_kv, A_w_q, A_w_uk, A_w_uv, A_w_o, B_x, B_w_r, B_w_gate, B_w_up, B_w_down, grad_out):
    return _impl(A_x, A_c_kv, A_w_q, A_w_uk, A_w_uv, A_w_o, B_x, B_w_r, B_w_gate, B_w_up, B_w_down, grad_out)
```

```python
import contextlib, math
import jax, jax.numpy as jnp
from jax import lax
import jax.experimental.pallas as pl
import jax.experimental.pallas.tpu as pltpu

S, M, H, D, DC, F, C = 2048, 576, 32, 128, 512, 4608, 8
T = 128
NB = S // T
NP = NB // 2
FC = 256
NFC = F // FC
CP = 16
G = 8
NG = H // G
f32, bf16, u32, i32 = jnp.float32, jnp.bfloat16, jnp.uint32, jnp.int32
LOG2E = math.log2(math.e)
LN2 = math.log(2.0)
SCALE = D ** -0.5
QSCALE = SCALE * LOG2E
EPS_B = 1.0013580322265625e-05
WROWS = (M, DC, DC)
MH = M // 2
CH = DC // 2
V = pltpu.VMEM
al = slice(None)

def nn(a, b): return lax.dot_general(a, b, (((1,), (0,)), ((), ())), preferred_element_type=f32)
def nt(a, b): return lax.dot_general(a, b, (((1,), (1,)), ((), ())), preferred_element_type=f32)
_nn, _nt = nn, nt
def rb(x): return x.astype(bf16).astype(f32)
def sigmoid_b(x): return rb(1.0 / rb(1.0 + rb(jnp.exp(-x))))
def sl(a, b): return slice(a * T, b * T)
def pk(x): return pltpu.bitcast(x.astype(bf16), u32)
def up(x): return pltpu.bitcast(x, bf16)
def cat(xs, axis): return xs[0] if len(xs) == 1 else jnp.concatenate(xs, axis=axis)

class Pk:
    def __init__(self, ref, col=None):
        self.ref, self.col = ref, col
        self.shape = (ref.shape[0] * 2, ref.shape[1])
    def _ix(self, idx):
        r, c = (al, al) if idx is Ellipsis else idx
        if self.col is not None:
            assert c == al
            c = sl(self.col, self.col + 1)
        r0 = 0 if r.start is None else r.start
        r1 = self.shape[0] if r.stop is None else r.stop
        assert r0 % 16 == 0 and r1 % 16 == 0
        return (slice(r0 // 2, r1 // 2), c)
    def __getitem__(self, idx):
        return up(self.ref[self._ix(idx)])
    def __setitem__(self, idx, val):
        self.ref[self._ix(idx)] = pk(val)

def PkV(r, c): return pltpu.VMEM((r // 2, c), u32)

NPT = 136 + 5 * 28
NDT = 136 + 5 * 28
SCR = dict(
    st_x=V((M, S), bf16), st_go=V((M, S), bf16), st_c=V((S, DC), bf16),
    wi0=V((M, G, D), bf16), wi1=V((DC, G, D), bf16), wi2=V((DC, G, D), bf16),
    wo0=V((M, G, D), bf16), wo1=V((DC, G, D), bf16), wo2=V((DC, G, D), bf16),
    wf0=V((2 * M * 4, D), u32), wf1=V((2 * DC * 4, D), u32), wf2=V((2 * DC * 4, D), u32),
    df0=V((3 * M * 4, D), u32), df12=V((2 * 2 * DC * 4, D), u32),
    woi=V((2, M, D), bf16), woo=V((4, M, D), bf16),
    mi=V((2, 3, M, FC), bf16), mo=V((2, 3, M, FC), bf16),
    xnT=PkV(M, S), goH=PkV(64, S), cT=PkV(DC, S), rstd=V((1, S), f32), wrb=V((M, T), f32), r=V((8, 256), f32),
    acc=V((2, M, S), f32), dcT=V((DC, S), f32),
    bm=V((2, 7, MH // 2, S // 2), u32), bc=V((7, CH // 2, S // 2), u32),
    oh=V((CP, S), bf16), xsel=V((CP, M), bf16), xselT=V((M, CP), bf16), gosel=V((CP, M), f32),
    dy=V((CP, M), bf16), dyT=V((M, CP), bf16), rs=V((CP, 128), f32), y=V((CP, M), f32), dxsel=V((CP, M), f32),
    wqT=PkV(D, 640), wo=PkV(D, 640), wkT=PkV(D, DC), wvT=PkV(D, DC), uo=PkV(7 * 64, 256), uv=PkV(7 * 64, 256),
    wm=V((2, 2, M, D), f32), wc=V((2, 2, DC, D), f32), em=V((2, 2, D, S), f32), ec=V((2, 2, D, S), f32),
    umc=PkV(7 * MH, 2 * D), cm=PkV(7 * D, S // 2), cc=PkV(7 * D, S // 2),
    dwm=V((4 * MH, D), f32), dwc=V((4 * CH, D), f32),
    qT=PkV(D, S), oT=PkV(D, S), kT=PkV(D, S), vT=PkV(D, S), kv=PkV(S, 2 * D),
    qc=PkV(7 * 64, S // 2), oc=PkV(7 * 64, S // 2), kc=PkV(7 * 64, S // 2), vc=PkV(7 * 64, S // 2),
    sT=V((136 * T, T), f32), pd=PkV(NPT * T, 2 * T), ml=V((136 * 8, 2 * T), f32),
    sem=pltpu.SemaphoreType.DMA((32,)),
)
PACKED = ("xnT", "goH", "cT", "wqT", "wo", "wkT", "wvT", "uo", "uv", "cm", "cc",
          "qT", "oT", "kT", "vT", "qc", "oc", "kc", "vc")
VIEWS = dict(um=("umc", 0), uc=("umc", 1), k=("kv", 0), v=("kv", 1), PT=("pd", 0), dST=("pd", 1))
PIN = ("wqT", "wo", "wvT", "uo", "uv", "umc", "cm", "cc", "dwm", "dwc",
       "qT", "oT", "kT", "vT", "kv", "qc", "oc", "kc", "vc", "sT", "pd", "ml")

SU = (((1, 0, 0), (1, 1, 1)), ((1, 1, 0), (1, 1, 1)), ((1, 0, 0),), ((1, 1, 1),), ((1, 0, 0), (1, 0, 1)),
      ((1, 1, 0), (-1, 0, 0)), ((1, 0, 1), (-1, 1, 1)))
SV = (((1, 0, 0), (1, 1, 1)), ((1, 0, 0),), ((1, 0, 1), (-1, 1, 1)), ((1, 1, 0), (-1, 0, 0)), ((1, 1, 1),),
      ((1, 0, 0), (1, 0, 1)), ((1, 1, 0), (1, 1, 1)))
SW = (((1, 0, 0), (1, 1, 1)), ((1, 1, 0), (-1, 1, 1)), ((1, 0, 1), (1, 1, 1)), ((1, 0, 0), (1, 1, 0)),
      ((1, 0, 1), (-1, 0, 0)), ((1, 1, 1),), ((1, 0, 0),))
IJ = ((0, 0), (0, 1), (1, 0), (1, 1))

def combo(terms, blk):
    (_, i, j) = terms[0]
    x = blk[i, j]
    if len(terms) == 2:
        sg, i, j = terms[1]
        x = x + blk[i, j] if sg > 0 else x - blk[i, j]
    return x

def scatter(table, prods, init=None):
    out = {} if init is None else {(i, j): (1, init[64 * i:64 * i + 64, j * T:(j + 1) * T]) for i, j in IJ}
    for r, x in prods.items():
        for sg, i, j in table[r]:
            if (i, j) not in out: out[i, j] = (sg, x)
            else:
                s0, y = out[i, j]
                out[i, j] = (s0, y + x) if s0 == sg else ((1, y - x) if s0 > 0 else (1, x - y))
    return out

def join(z):
    assert all(z[k][0] > 0 for k in IJ)
    return jnp.concatenate([jnp.concatenate([z[0, 0][1], z[0, 1][1]], axis=1),
                            jnp.concatenate([z[1, 0][1], z[1, 1][1]], axis=1)], axis=0)

def tile_id(t, j): return j * (j + 1) // 2 + t
def combo_id(r, a, b):
    if len(SV[r]) == 1:
        _, i, j = SV[r][0]
        return tile_id(2 * a + i, 2 * b + j)
    return 136 + 5 * (b * (b - 1) // 2) + (0, None, 1, 2, None, 3, 4)[r] * b + a

ORD7 = ("K0 K1 K2 K3 Q3 Q2 A3 A2 Xa3:A2:A2 V0 V1 V2 V3 O3 Q1 Xb3:V0:Q1 Xa2:V0:Q1 A1 B3 O2 Q0 Xb2:B3:Q0 Xa1:B3:Q0 A0 B2 O1 O0 PF "
        "Xb1:B2:O0 Xa0:B2:B2 Xb0:O1:O0 C3 B1 B0 D3 C2 EV3 EK3 EV2 D2 C1 EK2 C0 EV1 D1 D0 EK1 EV0 EK0")

ORD8 = ("K0 K1 K2 K3 Q3 V0 A3 V1 V2 V3 Q2 Xa3:V1:Q2 O3 O2 Q1 O1 Q0 O0 Xb3:O3:O0 A2 B3 Xa2:B3:B3 A1 C3 EV3 A0 D3 "
        "Xb2:EV3:D3 Xa1:EV3:D3 EK3 B2 EV2 PF Xb1:B2:EV2 Xa0:B2:EV2 C2 B1 D2 Xb0:B1:D2 C1 EK2 B0 EV1 D1 C0 EK1 D0 EV0 EK0")

ORD9 = ("K0 K1 K2 K3 Q3 V0 A3 V1 V2 V3 Q2 Xa3:V1:Q2 O3 O2 Q1 O1 Q0 O0 Xb3:O3:O0 A2 B3 Xa2:B3:B3 A1 C3 EV3 A0 D3 "
        "Xb2:EV3+200:D3 Xa1:EV3+200:D3 EK3 B2 EV2 Xb1:B2:EV2 Xa0:B2:EV2 C2 B1 D2 Xb0:B1+200:D2 C1 EK2 B0 EV1 D1 C0 EK1 D0 EV0 PF0:EK1:EV0 EK0")


class NS:
    def __init__(self, d):
        self._d = d
    def __getattr__(self, n):
        return self._d[n]


def make(cfg):
    names = list(SCR)
    scope = jax.named_scope if cfg.get('scopes') else (lambda n: contextlib.nullcontext())

    def kernel(xT_h, c_h, goT_h, wq_h, wuk_h, wuv_h, woT_h, wr_ref, wg_h, wu_h, wdT_h,
               outT_h, dxT_h, dc_h, dwq_h, dwuk_h, dwuv_h, dwoT_h, dwr_ref, dwg_h, dwu_h, dwdT_h, *scr):
        raw = dict(zip(names, scr))
        s = NS({**{n: Pk(raw[n]) if n in PACKED else raw[n] for n in names},
                **{n: Pk(raw[b], c_) for n, (b, c_) in VIEWS.items()}})
        sem = s.sem
        w_h = (wq_h, wuk_h, wuv_h); dw_h = (dwq_h, dwuk_h, dwuv_h)
        wi = (s.wi0, s.wi1, s.wi2); wo = (s.wo0, s.wo1, s.wo2)
        wf = (s.wf0, s.wf1, s.wf2)
        df = ((s.df0, 0), (s.df12, 2 * DC * 4), (s.df12, 0))
        m_h = (wg_h, wu_h, wdT_h); dm_h = (dwg_h, dwu_h, dwdT_h)
        cp = pltpu.make_async_copy
        XW = 512; NX = S // XW
        def ch(b): return pl.ds(pl.multiple_of(b * XW, XW), XW)

        def x_in(b): return cp(xT_h.at[:, ch(b)], s.st_x.at[:, ch(b)], sem.at[16 + b])
        def go_in(b): return cp(goT_h.at[:, ch(b)], s.st_go.at[:, ch(b)], sem.at[20 + b])
        def c_in(b): return cp(c_h.at[ch(b), :], s.st_c.at[ch(b), :], sem.at[24 + b])
        def o_x(b): return cp(s.st_x.at[:, ch(b)], outT_h.at[:, ch(b)], sem.at[16 + b])
        def o_go(b): return cp(s.st_go.at[:, ch(b)], dxT_h.at[:, ch(b)], sem.at[20 + b])
        def o_c(b): return cp(s.st_c.at[ch(b), :], dc_h.at[ch(b), :], sem.at[24 + b])
        def w_in_full(w): return cp(w_h[w].at[:, pl.ds(0, G), :], wi[w], sem.at[w])
        def w_in(w, t):
            n = WROWS[w] // G
            g = jnp.minimum((t >> 3) + 1, NG - 1)
            r = pl.ds((t & 7) * n, n)
            return cp(w_h[w].at[r, pl.ds(pl.multiple_of(g * G, G), G), :], wi[w].at[r], sem.at[w])
        def w_out(w, t):
            n = WROWS[w] // G
            g = jnp.maximum((t >> 3) - 1, 0)
            r = pl.ds((t & 7) * n, n)
            return cp(wo[w].at[r], dw_h[w].at[r, pl.ds(pl.multiple_of(g * G, G), G), :], sem.at[3 + w])
        def w_out_full(w): return cp(wo[w], dw_h[w].at[:, pl.ds((NG - 1) * G, G), :], sem.at[3 + w])
        def wo_in(t): return cp(woT_h.at[jnp.minimum(t, H - 1)], s.woi.at[t & 1], sem.at[6])
        def wo_out(p): return cp(s.woo.at[pl.ds(0, 2)], dwoT_h.at[pl.ds(2 * p, 2)], sem.at[7])
        def m_in(w, t): return cp(m_h[w].at[:, pl.ds(pl.multiple_of(t * FC, FC), FC)], s.mi.at[t & 1, w], sem.at[8 + w])
        def m_out(w, t): return cp(s.mo.at[t & 1, w], dm_h[w].at[:, pl.ds(pl.multiple_of(t * FC, FC), FC)], sem.at[11 + w])

        def cvt_in(w, slot, sl_, hold=lambda x: x):
            n = WROWS[w] // G
            x = wi[w][pl.ds(sl_ * n, n)].reshape(n * G, D)
            wf[w][pl.ds(pl.multiple_of(slot * (WROWS[w] * 4) + sl_ * (n * 4), 8), n * 4), :] = hold(pltpu.bitcast(x, u32))
        def cvt_out(w, slot, sl_, hold=lambda x: x):
            n = WROWS[w] // G
            x = df[w][0][pl.ds(pl.multiple_of(df[w][1] + slot * (WROWS[w] * 4) + sl_ * (n * 4), 8), n * 4), :]
            wo[w][pl.ds(sl_ * n, n)] = up(hold(x)).reshape(n, G, D)
        def w_load(w, h):
            x = wf[w][pl.ds(((h >> 3) & 1) * (WROWS[w] * 4) + ((h & 7) >> 1), WROWS[w], stride=4), :]
            sh = jnp.asarray(16 * (1 - (h & 1)), i32).astype(u32)
            return pltpu.bitcast((x << sh) & jnp.uint32(0xFFFF0000), f32)

        for b in range(NX): x_in(b).start()
        for b in range(NX):
            go_in(b).start(); c_in(b).start()
        for w in (1, 0, 2): w_in_full(w).start()
        wo_in(0).start()
        for w in range(3): m_in(w, 0).start()

        s.wrb[...] = jnp.broadcast_to(wr_ref[...].astype(f32), (T, M)).T

        def m_combos(kind, x, cn):
            for lo, n_, o in ((0, 256, 256), (512, 32, 32)):
                blk = {(i, j): x[j][lo + o * i:lo + o * i + n_] for i, j in IJ}
                d0 = min(lo, 256) // 2
                for r in range(7):
                    s.bm[kind, r, d0:d0 + n_ // 2, cn] = pk(combo(SV[r], blk))

        with scope("ln"):
            @pl.loop(0, NP)
            def _(n):
                @pl.when((n & 1) == 0)
                def _():
                    x_in(n >> 1).wait()
                xs = []; rs_ = []
                for j in range(2):
                    cs = pl.ds(pl.multiple_of(n * (2 * T) + j * T, T), T)
                    x = s.st_x[:, cs].astype(f32)
                    mu = jnp.mean(x, axis=0, keepdims=True)
                    xc32 = x - mu
                    var = jnp.mean(xc32 * xc32, axis=0, keepdims=True)
                    sd = rb(jnp.sqrt(rb(rb(var) + EPS_B)))
                    s.xnT[al, cs] = rb(x - rb(mu)) / sd
                    s.rstd[:, cs] = 1.0 / sd
                    xn = s.xnT[al, cs].astype(f32)
                    xs.append(xn)
                    rs_.append(jnp.sum(xn * s.wrb[...], axis=0, keepdims=True))
                s.r[pl.ds(n, 1), :] = rb(jnp.concatenate(rs_, axis=1))
                m_combos(1, xs, pl.ds(pl.multiple_of(n * T, T), T))
                for nm in PIN:
                    raw[nm][pl.ds(pl.multiple_of((n & 1) * 8, 8), 8), 0:128] = jnp.zeros((8, 128), raw[nm].dtype)

        col = (lax.broadcasted_iota(i32, (8, 256), 0) * 256 + lax.broadcasted_iota(i32, (8, 256), 1)).astype(f32)
        row = lax.broadcasted_iota(i32, (CP, T), 0)

        def goc(n, carry):
            r, idxs, rsel = carry
            @pl.when((n & 1) == 0)
            def _():
                go_in(n >> 1).wait(); c_in(n >> 1).wait()
            mx = jnp.max(jnp.max(r, axis=0, keepdims=True), axis=1, keepdims=True)
            ix = jnp.min(jnp.min(jnp.where(r == mx, col, float(S)), axis=0, keepdims=True), axis=1, keepdims=True)
            r = jnp.where(col == ix, -jnp.inf, r)
            idxs = jnp.where(row == n, ix, idxs)
            rsel = jnp.where(row == n, mx, rsel)
            cn = pl.ds(pl.multiple_of(n * T, T), T)
            gs = []; cs_ = []
            for j in range(2):
                cs = pl.ds(pl.multiple_of(n * (2 * T) + j * T, T), T)
                go = s.st_go[:, cs]
                s.goH[al, cs] = go[512:M]
                gs.append(go.astype(f32))
                s.cT[al, cs] = s.st_c[cs, :].T
                cs_.append(s.cT[al, cs].astype(f32))
            m_combos(0, gs, cn)
            blk = {(i, j): cs_[j][CH * i:CH * i + CH] for i, j in IJ}
            for q in range(7):
                s.bc[q, :, cn] = pk(combo(SV[q], blk))
            return r, idxs, rsel
        with scope("goc"):
            _, idxs, rsel = lax.fori_loop(0, NP, goc, (s.r[...], jnp.full((CP, T), -1.0, f32), jnp.zeros((CP, T), f32)))

        with scope("gather"):
            colf = lax.broadcasted_iota(i32, (CP, S), 1).astype(f32)
            s.oh[...] = jnp.where(colf == idxs[:, 0:1], 1.0, 0.0).astype(bf16)
            s.rs[...] = sigmoid_b(rsel)
            s.y[...] = jnp.zeros_like(s.y)
            s.gosel[...] = jnp.zeros_like(s.gosel)
            s.dxsel[...] = jnp.zeros_like(s.dxsel)
            @pl.loop(0, NX)
            def _(b):
                s.y[...] += nt(s.oh[:, ch(b)], s.xnT[al, ch(b)])
                s.gosel[...] += nt(s.oh[:, ch(b)], s.st_go[:, ch(b)])
            xsel = s.y[...]
            s.xsel[...] = xsel.astype(bf16)
            dy = s.gosel[...] * s.rs[:, 0:1]
            s.dy[...] = dy.astype(bf16)
            s.xselT[...] = xsel.T.astype(bf16)
            s.dyT[...] = dy.T.astype(bf16)
            s.y[...] = jnp.zeros_like(s.y)

        with scope("wcvt"):
            for w in range(3): w_in_full(w).wait()
            @pl.loop(0, G + 1)
            def _(i):
                @pl.when(i == G)
                def _():
                    for w in range(3): w_in(w, 0).wait()
                    for w in range(3): w_in(w, 1).start()
                for w in range(3): cvt_in(w, i >> 3, i & 7)
                @pl.when(i == 0)
                def _():
                    for w in range(3): w_in(w, 0).start()
            s.wkT[...] = w_load(1, 0).astype(bf16).T

        def main_step(h):
            g = h >> 3
            odd = h & 1
            for w in range(3): w_in(w, h + 1).wait()
            wo_in(h).wait()
            @pl.when(h >= G + 2)
            def _():
                for w in range(3): w_out(w, h - 2).wait()
            @pl.when(jnp.logical_and(h >= 3, odd == 1))
            def _():
                wo_out((h >> 1) - 1).wait()
            for w in range(3): w_in(w, h + 2).start()
            wo_in(h + 1).start()
            @pl.when(h >= G + 1)
            def _():
                for w in range(3): w_out(w, h - 1).start()
            @pl.when(jnp.logical_and(h >= 2, odd == 0))
            def _():
                wo_out((h >> 1) - 1).start()

            @pl.when(h < NFC)
            def _moe():
                for w in range(3): m_in(w, h).wait()
                @pl.when(h + 1 < NFC)
                def _():
                    for w in range(3): m_in(w, h + 1).start()
                @pl.when(h >= 1)
                def _():
                    for w in range(3): m_out(w, h - 1).wait()
                wg = s.mi[odd, 0]; wu = s.mi[odd, 1]; wdT = s.mi[odd, 2]
                xs = s.xsel[...]
                a = rb(nn(xs, wg)); u = rb(nn(xs, wu))
                dh = rb(nn(s.dy[...], wdT))
                sg = sigmoid_b(a)
                g_ = rb(a * sg)
                hb = (g_ * u).astype(bf16)
                dg = rb(dh * u)
                da = (rb(dg * sg) + rb(rb(a * dg) * rb(sg * (1.0 - sg)))).astype(bf16)
                du = (dh * g_).astype(bf16)
                s.y[...] += nt(hb, wdT)
                s.dxsel[...] += nt(da, wg) + nt(du, wu)
                s.mo[odd, 0] = nn(s.xselT[...], da).astype(bf16)
                s.mo[odd, 1] = nn(s.xselT[...], du).astype(bf16)
                s.mo[odd, 2] = nn(s.dyT[...], hb).astype(bf16)
                for w in range(3): m_out(w, h).start()

            def side(hold):
                for w in range(3): cvt_in(w, (((h + 1) >> 3) + 1) & 1, (h + 1) & 7, hold)
                for w in range(3): cvt_out(w, (g + 1) & 1, h & 7, hold)
            with scope('headA'):
                head_body(cfg, s, h, w_load, side)

            @pl.when(odd == 1)
            def _():
                if cfg.get("unrollP"):
                    with scope('pairP'):
                        for kind in range(2):
                            pair_body(cfg, s, kind, h)
                else:
                    @pl.loop(0, 2)
                    def _(kind):
                        with scope('pairP'):
                            pair_body(cfg, s, kind, h)

        with scope('main'):
            pl.loop(0, H)(main_step)

        for w in range(3): w_in(w, H + 1).wait()
        wo_in(H).wait()
        for w in range(3): w_out(w, H - 2).wait()
        for w in range(3): w_out(w, H - 1).start()
        wo_out(H // 2 - 1).start()
        for w in range(3): m_out(w, NFC - 1).wait()

        rs = s.rs[:, 0:1]
        y = rb(s.y[...])
        drs = rb(jnp.sum(rb(s.gosel[...] * y), axis=1, keepdims=True))
        dr = rb(drs * rb(rs * (1.0 - rs)))
        wr = wr_ref[...].astype(f32)
        dwr_ref[...] = jnp.sum(dr * s.xsel[...].astype(f32), axis=0, keepdims=True).astype(bf16)
        s.xselT[...] = (y * rs).T.astype(bf16)
        s.dyT[...] = (s.dxsel[...] + dr * wr).T.astype(bf16)

        for w in range(3): w_out(w, H - 1).wait()
        @pl.loop(0, G)
        def _(i):
            for w in range(3): cvt_out(w, (NG - 1) & 1, i)
        for w in range(3): w_out_full(w).start()

        with scope("fin"):
            @pl.loop(0, NX)
            def _(bb):
                @pl.loop(0, XW // T)
                def _(b4):
                    cs = pl.ds(pl.multiple_of((bb * (XW // T) + b4) * T, T), T)
                    s.st_c[cs, :] = s.dcT[:, cs].astype(bf16).T
                    oh = s.oh[:, cs]
                    xn = s.xnT[al, cs].astype(f32)
                    s.st_x[:, cs] = (s.st_x[:, cs].astype(f32) + xn + s.acc[0, :, cs] + nn(s.xselT[...], oh)).astype(bf16)
                    go = s.st_go[:, cs].astype(f32)
                    dxn = s.acc[1, :, cs] + go + nn(s.dyT[...], oh)
                    m1 = jnp.mean(dxn, axis=0, keepdims=True)
                    m2 = jnp.mean(dxn * xn, axis=0, keepdims=True)
                    s.st_go[:, cs] = (go + s.rstd[:, cs] * (dxn - m1 - xn * m2)).astype(bf16)
                o_c(bb).start()
                o_x(bb).start()
                o_go(bb).start()
        for b in range(NX):
            o_c(b).wait(); o_x(b).wait(); o_go(b).wait()
        for w in range(3): w_out_full(w).wait()
        wo_out(H // 2 - 1).wait()

    def fn(A_x, A_c_kv, A_w_q, A_w_uk, A_w_uv, A_w_o, B_x, B_w_r, B_w_gate, B_w_up, B_w_down, grad_out):
        xT = A_x.reshape(S, M).T; goT = grad_out.reshape(S, M).T; c = A_c_kv.reshape(S, DC)
        woT = jnp.swapaxes(A_w_o, 1, 2)
        wr = B_w_r.reshape(1, M)
        wdT = B_w_down.T
        sds = jax.ShapeDtypeStruct
        hbm = pl.BlockSpec(memory_space=pl.ANY)
        vm = pl.BlockSpec(memory_space=pltpu.VMEM)
        outs = pl.pallas_call(
            kernel,
            in_specs=[hbm] * 7 + [vm] + [hbm] * 3,
            out_specs=[hbm] * 7 + [vm] + [hbm] * 3,
            out_shape=[sds((M, S), bf16), sds((M, S), bf16), sds((S, DC), bf16), sds((M, H, D), bf16),
                       sds((DC, H, D), bf16), sds((DC, H, D), bf16), sds((H, M, D), bf16), sds((1, M), bf16),
                       sds((M, F), bf16), sds((M, F), bf16), sds((M, F), bf16)],
            scratch_shapes=list(SCR.values()),
            compiler_params=pltpu.CompilerParams(vmem_limit_bytes=124 * 1024 * 1024),
            name="mla",
        )(xT, c, goT, A_w_q, A_w_uk, A_w_uv, woT, wr, B_w_gate, B_w_up, wdT)
        outT, dxT, dc, dwq, dwuk, dwuv, dwoT, dwr, dwg, dwu, dwdT = outs
        return (outT.T.reshape(1, S, M), dxT.T.reshape(1, S, M), dc.reshape(1, S, DC), dwq, dwuk, dwuv,
                jnp.swapaxes(dwoT, 1, 2), dwr.reshape(M), dwg, dwu, dwdT.T)
    return fn


def head_body(cfg, s, h, w_load, side):
    tri = lax.broadcasted_iota(i32, (T, T), 0) <= lax.broadcasted_iota(i32, (T, T), 1)
    never = lax.broadcasted_iota(i32, (8, T), 0) + h < 0
    st = {}
    order = cfg.get("order", ORD7)
    sB, sD = cfg.get("sB", 1), cfg.get("sD", 1)
    hs = h & 1
    toks = []; span = {}

    def tree(op, xs):
        xs = list(xs)
        while len(xs) > 1:
            xs = [op(xs[i], xs[i + 1]) if i + 1 < len(xs) else xs[i] for i in range(0, len(xs), 2)]
        return xs[0]
    def vregs(x):
        return [x[8 * i:8 * i + 8, :] for i in range(x.shape[0] // 8)]
    load = [0, 0, 0, 0]
    def track(x, k):
        for c in range(x.shape[1] // T):
            t0 = 0
            for _ in range(-(-k // T)):
                q = load.index(min(load))
                t0 = max(t0, load[q])
                load[q] += x.shape[0]
            for i in range(x.shape[0] // 8):
                toks.append((t0 + 8 * i, x, i, c))
        return x
    def nn(a, b): return track(_nn(a, b), a.shape[1])
    def nt(a, b): return track(_nt(a, b), a.shape[1])
    class Gate:
        def __init__(self, a, b, n):
            a, _, sk = a.partition("+"); b, _, tl = b.partition("-")
            self.t0 = span[a][0] + int(sk or cfg.get("skip", 64)); self.t1 = span[b][1] - int(tl or cfg.get("tail", 64))
            self.n, self.g = n, 0
        def next(self):
            t = self.t0 + (self.t1 - self.t0) * self.g / self.n
            _, x, i, c = min(toks, key=lambda e: abs(e[0] - t))
            self.g += 1
            return x[8 * i:8 * i + 8, c * T:(c + 1) * T]
        def hold(self, x):
            n = x.shape[0] // 8
            tk = self.next()
            if x.dtype != f32: tk = pltpu.bitcast(tk, x.dtype)
            return jnp.where(never[None], tk[None], x.reshape(n, 8, T)).reshape(n * 8, T)
    def rows(i, lo=0, hi=T): return slice(i * T + lo, i * T + hi)
    def exp_rows(x, m):
        n = x.shape[0] // 8
        return jnp.exp2(x.reshape(n, 8, T) - m[None]).reshape(n * 8, T)

    def W():
        s.wc[1, hs] = w_load(1, h)
        wq = w_load(0, h); s.wm[1, hs] = wq
        s.wqT[al, :M] = wq.astype(bf16).T
        woT = s.woi[hs]; s.wm[0, hs] = woT.astype(f32)
        s.wo[al, :M] = woT.T
        wv = w_load(2, h); s.wc[0, hs] = wv
        s.wvT[...] = wv.astype(bf16).T
        for src, dst in ((s.wo, s.uo), (s.wvT, s.uv)):
            blk = {(i, j): src[slice(64 * i, 64 * i + 64), slice(256 * j, 256 * j + 256)].astype(f32) for i, j in IJ}
            for r in range(7):
                dst[slice(64 * r, 64 * r + 64), al] = combo(SU[r], blk)
    def fwd(u, b, init=None):
        return join(scatter(SW, {r: (nn(u[slice(64 * r, 64 * r + 64), al], up(b(r)))) for r in range(7)}, init))
    def put(z, n, xT, xc, table, on):
        xT[al, sl(2 * n, 2 * n + 2)] = z
        if on:
            blk = {(i, j): z[64 * i:64 * i + 64, j * T:(j + 1) * T] for i, j in IJ}
            for r in range(7):
                xc[slice(64 * r, 64 * r + 64), sl(n, n + 1)] = combo(table[r], blk)
    def K(J):
        z = (nn(s.wkT[...], s.cT[al, sl(4 * J, 4 * J + 4)]))
        for n in range(2 * J, 2 * J + 2):
            put(z[:, sl(2 * n - 4 * J, 2 * n - 4 * J + 2)], n, s.kT, s.kc, SU, sD and n < NP - 1)
        s.k[sl(4 * J, 4 * J + 4), al] = s.kT[al, sl(4 * J, 4 * J + 4)].T
    def Q(J):
        z = (nn(s.wqT[al, :M], s.xnT[al, sl(4 * J, 4 * J + 4)])) * QSCALE
        for n in range(2 * J, 2 * J + 2):
            put(z[:, sl(2 * n - 4 * J, 2 * n - 4 * J + 2)], n, s.qT, s.qc, SW, sD and n > 0)
    def Vv(J):
        for n in range(2 * J, 2 * J + 2):
            put(fwd(s.uv, lambda q: s.bc[q, :, sl(n, n + 1)]), n, s.vT, s.vc, SU, sB and n < NP - 1)
            x = [pltpu.bitcast(s.vT[al, sl(2 * n + j, 2 * n + j + 1)].T, u32).reshape(8, 1, 8, T) for j in range(2)]
            s.kv[n * T:(n + 1) * T, T:] = jnp.concatenate(x, axis=1).reshape(T, T)
    def O(J):
        for n in range(2 * J, 2 * J + 2):
            hi = nn(s.wo[al, 512:M], s.goH[al, sl(2 * n, 2 * n + 2)])
            put(fwd(s.uo, lambda q: s.bm[0, q, 0:128, sl(n, n + 1)], hi), n, s.oT, s.oc, SW, sB and n > 0)
    def A(J):
        for j in range(4 * J + 3, 4 * J - 1, -1):
            x = nn(s.k[sl(0, j + 1), al], s.qT[al, sl(j, j + 1)])
            sd = jnp.where(tri, x[j * T:, :], -1e9)
            x = sd if j == 0 else jnp.concatenate([x[:j * T, :], sd], axis=0)
            for t in range(j + 1):
                vs = vregs(x[t * T:(t + 1) * T]); a = vs[0]
                for y in vs[1:]:
                    a = jnp.maximum(a, y)
                s.ml[tile_id(t, j) * 8:tile_id(t, j) * 8 + 8, :T] = a
            a = s.ml[tile_id(0, j) * 8:tile_id(j, j) * 8 + 8, :T]
            st["m", j] = jnp.broadcast_to(jnp.max(a, axis=0, keepdims=True), (8, T))
            s.sT[sl(tile_id(0, j), tile_id(j, j) + 1), :] = x
    def Xa(J, wa, wb):
        GA = cfg.get("GA", 128)
        gate = Gate(wa, wb, (16 * J + 10) * (T // GA))
        for j in range(4 * J, 4 * J + 4):
            m = st["m", j]
            for t in range(j + 1):
                s_ = None
                for lo in range(0, T, GA):
                    m = jnp.where(never, gate.next(), m)
                    y = tree(jnp.add, vregs(exp_rows(s.sT[rows(tile_id(t, j), lo, lo + GA), :], m)))
                    s_ = y if s_ is None else s_ + y
                s.ml[tile_id(t, j) * 8:tile_id(t, j) * 8 + 8, T:] = s_
            l = s.ml[tile_id(0, j) * 8:tile_id(j, j) * 8 + 8, T:]
            st["c", j] = m + jnp.log2(jnp.sum(l, axis=0, keepdims=True))
    def Xb(J, wa, wb):
        GB = cfg.get("GB", 32)
        gate = Gate(wa, wb, (16 * J + 10) * (32 // GB))
        for b in (2 * J + 1, 2 * J):
            c = [st["c", 2 * b], st["c", 2 * b + 1]]
            for a in range(b):
                for lo in range(0, T, GB):
                    tk = gate.next()
                    c = [jnp.where(never, tk, x) for x in c]
                    blk = {(i, j): exp_rows(s.sT[rows(tile_id(2 * a + i, 2 * b + j), lo, lo + GB), :], c[j]) for i, j in IJ}
                    for i, j in IJ:
                        s.PT[rows(tile_id(2 * a + i, 2 * b + j), lo, lo + GB), al] = blk[i, j]
                    if sB:
                        for r in range(7):
                            if len(SV[r]) == 2:
                                s.PT[rows(combo_id(r, a, b), lo, lo + GB), al] = combo(SV[r], blk)
            for i, j in ((0, 0), (0, 1), (1, 1)):
                for lo in range(0, T, 4 * GB):
                    c[j] = jnp.where(never, gate.next(), c[j])
                    ix = rows(tile_id(2 * b + i, 2 * b + j), lo, lo + 4 * GB)
                    s.PT[ix, al] = exp_rows(s.sT[ix, :], c[j])
    def left(Y, xT, xc, b, on):
        t0 = 2 * b if on else 0
        z = []
        for j in range(2):
            a = None
            for q0 in range(t0, 2 * b + j + 1, 4):
                q1 = min(q0 + 4, 2 * b + j + 1)
                x = (nn(xT[al, sl(q0, q1)], Y[sl(tile_id(q0, 2 * b + j), tile_id(q1 - 1, 2 * b + j) + 1), al]))
                a = x if a is None else a + x
            z.append(a)
        z = jnp.concatenate(z, axis=1)
        if on and b > 0:
            pr_ = {r: (nn(xc[slice(64 * r, 64 * r + 64), sl(0, b)],
                             cat([Y[rows(combo_id(r, a, b)), al] for a in range(b)], 0))) for r in range(7)}
            z = join(scatter(SW, pr_, z))
        return z
    def right(Y, xT, xc, a, on):
        t1 = 2 * a + 2 if on else NB
        z = [(nt(xT[al, sl(2 * a + i, t1)], cat([Y[rows(tile_id(2 * a + i, j)), al] for j in range(2 * a + i, t1)], 1)))
             for i in range(2)]
        z = jnp.concatenate(z, axis=1)
        if on and a < NP - 1:
            pr_ = {r: (nt(xc[slice(64 * r, 64 * r + 64), sl(a + 1, NP)],
                             cat([Y[rows(combo_id(r, a, b)), al] for b in range(a + 1, NP)], 1))) for r in range(7)}
            z = join(scatter(SU, pr_, z))
        return z
    def B(J):
        for b in (2 * J + 1, 2 * J):
            cs = sl(2 * b, 2 * b + 2)
            ctxT = left(s.PT, s.vT, s.vc, b, sB)
            st["dl", b] = jnp.sum(ctxT * s.oT[al, cs].astype(f32), axis=0, keepdims=True)
            s.em[0, hs, :, cs] = ctxT
    def Cc(J):
        dp = {}
        for b in (2 * J + 1, 2 * J):
            if b > 0:
                dp[b] = nn(s.v[sl(0, 2 * b), al], s.oT[al, sl(2 * b, 2 * b + 2)])
        for b in (2 * J + 1, 2 * J):
            vd = s.kv[b * T:(b + 1) * T, T:].reshape(8, 2, 8, T)
            dp[b, 1] = nn(s.v[sl(2 * b, 2 * b + 2), al], s.oT[al, sl(2 * b + 1, 2 * b + 2)])
            dp[b, 0] = nn(up(vd[:, 0].reshape(64, T)), s.oT[al, sl(2 * b, 2 * b + 1)])
        def ds(x, t, j, b):
            return s.PT[rows(tile_id(t, j)), al].astype(f32) * (x - st["dl", b][:, (j - 2 * b) * T:(j - 2 * b + 1) * T])
        def deint(x, i): return x.reshape(8, 2, 16, T)[:, i].reshape(T, T)
        for b in (2 * J + 1, 2 * J):
            for a in range(b):
                blk = {(i, j): ds(deint(dp[b][a * 2 * T:(a + 1) * 2 * T, j * T:(j + 1) * T], i), 2 * a + i, 2 * b + j, b) for i, j in IJ}
                if sD:
                    for r in range(7):
                        s.dST[rows(combo_id(r, a, b)), al] = combo(SV[r], blk)
                else:
                    for i, j in IJ:
                        s.dST[rows(tile_id(2 * a + i, 2 * b + j)), al] = blk[i, j]
            s.dST[rows(tile_id(2 * b, 2 * b)), al] = ds(dp[b, 0], 2 * b, 2 * b, b)
            for i in range(2):
                s.dST[rows(tile_id(2 * b + i, 2 * b + 1)), al] = ds(deint(dp[b, 1], i), 2 * b + i, 2 * b + 1, b)
    def Dd(J):
        for b in (2 * J + 1, 2 * J):
            s.em[1, hs, :, sl(2 * b, 2 * b + 2)] = left(s.dST, s.kT, s.kc, b, sD) * SCALE
    def EV(I):
        for a in (2 * I + 1, 2 * I):
            s.ec[0, hs, :, sl(2 * a, 2 * a + 2)] = right(s.PT, s.oT, s.oc, a, sB)
    def EK(I):
        for a in (2 * I + 1, 2 * I):
            s.ec[1, hs, :, sl(2 * a, 2 * a + 2)] = right(s.dST, s.qT, s.qc, a, sD) * LN2
    def PF(_, wa, wb):
        gate = Gate(wa, wb, 4 + 6 * 2)
        w = w_load(1, jnp.minimum(h + 1, H - 1))
        for c in range(DC // T):
            s.wkT[al, sl(c, c + 1)] = gate.hold(w[c * T:(c + 1) * T]).astype(bf16).T
        side(lambda x: cat([gate.hold(x[:x.shape[0] // 16 * 8]), gate.hold(x[x.shape[0] // 16 * 8:])], 0))
    ops = dict(K=K, V=Vv, Q=Q, O=O, A=A, Xa=Xa, Xb=Xb, B=B, C=Cc, D=Dd, EV=EV, EK=EK, PF=PF)
    W()
    for tk_ in order.split():
        name, *win = tk_.split(":")
        assert name not in span
        t0 = sum(load) // 4
        ops[name[:-1]](int(name[-1]), *win)
        span[name] = (t0, sum(load) // 4)
    assert len(span) == 4 * len(ops) - 3, len(span)


def pair_body(cfg, s, kind, h):
    slot = (h >> 3) & 1; pr = (h & 7) >> 1
    sides = dict(
        c=dict(R=CH, e=s.ec, w=s.wc, u=s.uc, cmb=s.cc, b=lambda r: s.bc[r], dw=s.dwc, acc=s.dcT, pre=(),
               first=jnp.logical_and(h == 1, kind == 0)),
        m=dict(R=MH, e=s.em, w=s.wm, u=s.um, cmb=s.cm, b=lambda r: s.bm[kind, r], dw=s.dwm, acc=s.acc, pre=(kind,),
               first=h == 1))
    for d in sides.values():
        for n in range(NP):
            blk = {(i, j): d["e"][kind, i, :, sl(2 * n + j, 2 * n + j + 1)] for i, j in IJ}
            for r in range(7):
                d["cmb"][sl(r, r + 1), sl(n, n + 1)] = combo(SW[r], blk)
        R = d["R"]
        blk = {(i, j): d["w"][kind, i, j * R:(j + 1) * R, :] for i, j in IJ}
        for r in range(7):
            d["u"][slice(r * R, (r + 1) * R), al] = combo(SU[r], blk)

    def wgrad(d):
        R = d["R"]; a_ref = d["dw"]
        done = set(); left = {}
        for r in range(7):
            for _, i, j in SU[r]: left[i, j] = left.get((i, j), 0) + 1
        fin = {}
        for r in range(7):
            x = nt(up(d["b"](r)), d["cmb"][sl(r, r + 1), al])
            for sg, i, j in SU[r]:
                ix = slice((2 * i + j) * R, (2 * i + j + 1) * R)
                if (i, j) not in done:
                    assert sg > 0
                    y = x
                else:
                    y = a_ref[ix, :] + x if sg > 0 else a_ref[ix, :] - x
                done.add((i, j)); left[i, j] -= 1
                if left[i, j]: a_ref[ix, :] = y
                else: fin[i, j] = y
        return fin
    def words(lo, hi):
        return (pltpu.bitcast(rb(lo), u32) >> 16) | pltpu.bitcast(rb(hi), u32)
    def DWC():
        fin = wgrad(sides["c"])
        base = kind * (2 * DC * 4) + slot * (DC * 4) + pr
        for j in range(2):
            s.df12[pl.ds(base + j * CH * 4, CH, stride=4), :] = words(fin[0, j], fin[1, j])
    def DWM():
        fin = wgrad(sides["m"])
        base = jnp.where(kind == 1, slot, 2) * (M * 4) + pr
        for j in range(2):
            w_ = words(fin[0, j], fin[1, j])
            s.df0[pl.ds(base + j * 256 * 4, 256, stride=4), :] = w_[:256]
            s.df0[pl.ds(base + (512 + 32 * j) * 4, 32, stride=4), :] = w_[256:]
            for i in range(2):
                s.woo[2 * kind + i, 256 * j:256 * j + 256, :] = fin[i, j][:256].astype(bf16)
                s.woo[2 * kind + i, 512 + 32 * j:544 + 32 * j, :] = fin[i, j][256:].astype(bf16)
    R1, R2 = (0, 1, 3, 5), (2, 4, 6)
    def BACK(d):
        R = d["R"]; acc = d["acc"]
        for q in range(2):
            a, b_, c_, e = range(4 * q, 4 * q + 4)
            for n, rs in ((a, R1), (b_, R1), (c_, R1), (e, R1), (a, R2), (e, (2,)), (b_, R2), (e, (4,)), (c_, R2), (e, (6,))):
                z = scatter(SV, {r: nn(d["u"][slice(r * R, (r + 1) * R), al], d["cmb"][sl(r, r + 1), sl(n, n + 1)]) for r in rs})
                for (i, j), (sg, x) in sorted(z.items()):
                    ix = d["pre"] + (slice(i * R, (i + 1) * R), sl(2 * n + j, 2 * n + j + 1))
                    old = acc[ix]
                    if rs is R1: old = jnp.where(d["first"], 0.0, old)
                    acc[ix] = old + x if sg > 0 else old - x
    for t in cfg.get("pord", "DWC DWM BC BM").split():
        dict(DWC=DWC, DWM=DWM, BC=lambda: BACK(sides["c"]), BM=lambda: BACK(sides["m"]))[t]()


_impl = make(dict(order=ORD9, GA=32, GB=16))


@jax.jit
def pallas_parallel_sum__compressed_kv_cla__moe_arch_mod__prompt_kernel(
        A_x, A_c_kv, A_w_q, A_w_uk, A_w_uv, A_w_o, B_x, B_w_r, B_w_gate, B_w_up, B_w_down, grad_out):
    return _impl(A_x, A_c_kv, A_w_q, A_w_uk, A_w_uv, A_w_o, B_x, B_w_r, B_w_gate, B_w_up, B_w_down, grad_out)
```

```python
import contextlib, math
import jax, jax.numpy as jnp
from jax import lax
import jax.experimental.pallas as pl
import jax.experimental.pallas.tpu as pltpu

S, M, H, D, DC, F, C = 2048, 576, 32, 128, 512, 4608, 8
T = 128
NB = S // T
NP = NB // 2
FT = 3
FC = FT * T
NFC = F // FC
CP = 16
f32, bf16, u32, i32 = jnp.float32, jnp.bfloat16, jnp.uint32, jnp.int32
LOG2E = math.log2(math.e)
LN2 = math.log(2.0)
SCALE = D ** -0.5
QSCALE = SCALE * LOG2E
EPS_B = 1.0013580322265625e-05
WROWS = (M, DC, DC)
WOFF = (0, M // 4, (M + DC) // 4)
WS = (M + 2 * DC) // 4
MQ = M // 4
SP = S + T
CH = DC // 2
V = pltpu.VMEM
al = slice(None)

def nn(a, b): return lax.dot_general(a, b, (((1,), (0,)), ((), ())), preferred_element_type=f32)
def nt(a, b): return lax.dot_general(a, b, (((1,), (1,)), ((), ())), preferred_element_type=f32)
def rb(x): return x.astype(bf16).astype(f32)
def sigmoid_b(x): return rb(1.0 / rb(1.0 + rb(jnp.exp(-x))))
def sl(a, b): return slice(a * T, b * T)
def pk(x): return pltpu.bitcast(x.astype(bf16), u32)
def up(x): return pltpu.bitcast(x, bf16)
def cat(xs, axis): return xs[0] if len(xs) == 1 else jnp.concatenate(xs, axis=axis)

class Pk:
    def __init__(self, ref, col=None, row0=0, rows=None):
        self.ref, self.col, self.row0 = ref, col, row0
        self.shape = (rows or ref.shape[0] * 2, ref.shape[1])
    def _ix(self, idx):
        r, c = (al, al) if idx is Ellipsis else idx
        if self.col is not None:
            assert c == al
            c = sl(self.col, self.col + 1)
        r0 = 0 if r.start is None else r.start
        r1 = self.shape[0] if r.stop is None else r.stop
        assert r0 % 16 == 0 and r1 % 16 == 0
        return (slice((self.row0 + r0) // 2, (self.row0 + r1) // 2), c)
    def __getitem__(self, idx):
        return up(self.ref[self._ix(idx)])
    def __setitem__(self, idx, val):
        self.ref[self._ix(idx)] = pk(val)

def PkV(r, c): return pltpu.VMEM((r // 2, c), u32)

NPT = 136 + 5 * 28
SCR = dict(
    st_x=V((NB, M, T), bf16), st_go=V((NB, M, T), bf16), st_c=V((4, S, T), bf16),
    wi=V((WS, 8, D), bf16), wkn=V((DC // 4 + 2, 8, D), bf16), wout=V((WS + 2, 8, D), bf16), woi=V((M, D), bf16), woo=V((2, M, D), bf16),
    mi=V((3 * FT + 2, M, T), bf16), mo=V((3 * FT, M, T), bf16), zero=V((CP, T), bf16), wr1=V((M,), bf16), wr=V((8, M), f32),
    goT=PkV(M, SP), xnT=PkV(M, SP), cT=PkV(DC, SP), stat=V((8, S), f32), wrb=V((M, T), f32), r=V((NB, T), f32), tok=pltpu.SMEM((C,), i32),
    acc=V((2, M, SP), f32), dcT=V((DC + T, SP), f32),
    bs=PkV(3 * 5 * CH, S // 2 + T), hz=PkV(3 * 14 * MQ, S // 4 + T),
    xb=V((2, C, M, T), f32),
    xsel=V((CP, M), bf16), gosel=V((CP, M), f32), dy=V((CP, M), bf16),
    upd=V((2 * CP, 5 * T), f32), mr=V((3 * FT * C, T), f32), rs=V((CP, 128), f32), y=V((CP, M), f32), dxsel=V((CP, M), f32),
    wqT=PkV(D, 640), wo=PkV(D, 640), wkT=PkV(D, DC), wvT=PkV(D, DC), uo=PkV(7 * 64, 256), uv=PkV(7 * 64, 256),
    uq=PkV(7 * 64, 256), uk=PkV(7 * 64, 256),
    wm=V((2, 2, M, D), f32), wc=V((2, 2, DC, D), f32), em=V((2, 2, D, SP), f32), ec=V((2, 2, D, SP), f32),
    qT=PkV(D, S), oT=PkV(D, S), kT=PkV(D, S), vT=PkV(D, S), kv=PkV(S, 2 * D),
    qc=PkV(7 * 64, S // 2), oc=PkV(7 * 64, S // 2), kc=PkV(7 * 64, S // 2), vc=PkV(7 * 64, S // 2),
    sT=V((136 * T, T), f32), pd=PkV(NPT * T, 2 * T), ml=V((136 * 8, 2 * T), f32),
    sem=pltpu.SemaphoreType.DMA((24,)),
)
PACKED = ("goT", "xnT", "cT", "bs", "hz", "wqT", "wo", "wkT", "wvT", "uo", "uv", "uq", "uk",
          "qT", "oT", "kT", "vT", "qc", "oc", "kc", "vc")
VIEWS = dict(k=("kv", 0), v=("kv", 1), PT=("pd", 0), dST=("pd", 1))
PIN = ("wqT", "wo", "wvT", "wkT", "uo", "uv", "uq",
       "qT", "oT", "kT", "vT", "kv", "qc", "oc", "kc", "vc", "sT", "pd", "ml")

SU = (((1, 0, 0), (1, 1, 1)), ((1, 1, 0), (1, 1, 1)), ((1, 0, 0),), ((1, 1, 1),), ((1, 0, 0), (1, 0, 1)),
      ((1, 1, 0), (-1, 0, 0)), ((1, 0, 1), (-1, 1, 1)))
SV = (((1, 0, 0), (1, 1, 1)), ((1, 0, 0),), ((1, 0, 1), (-1, 1, 1)), ((1, 1, 0), (-1, 0, 0)), ((1, 1, 1),),
      ((1, 0, 0), (1, 0, 1)), ((1, 1, 0), (1, 1, 1)))
SW = (((1, 0, 0), (1, 1, 1)), ((1, 1, 0), (-1, 1, 1)), ((1, 0, 1), (1, 1, 1)), ((1, 0, 0), (1, 1, 0)),
      ((1, 0, 1), (-1, 0, 0)), ((1, 1, 1),), ((1, 0, 0),))
IJ = ((0, 0), (0, 1), (1, 0), (1, 1))
R2 = (0, 2, 3, 5, 6)
HT = (-0.375, -1.5, 0.375, 1.5)
HP = ((0, 1), (0, 2), (0, 3), (1, 2), (1, 3), (2, 3))

def combo(terms, blk):
    (_, i, j) = terms[0]
    x = blk[i, j]
    if len(terms) == 2:
        sg, i, j = terms[1]
        x = x + blk[i, j] if sg > 0 else x - blk[i, j]
    return x

def scatter(table, prods, init=None):
    out = {} if init is None else {(i, j): (1, init[64 * i:64 * i + 64, j * T:(j + 1) * T]) for i, j in IJ}
    for r, x in prods.items():
        for sg, i, j in table[r]:
            if (i, j) not in out: out[i, j] = (sg, x)
            else:
                s0, y = out[i, j]
                out[i, j] = (s0, y + x) if s0 == sg else ((1, y - x) if s0 > 0 else (1, x - y))
    return out

def join(z):
    assert all(z[k][0] > 0 for k in IJ)
    return jnp.concatenate([jnp.concatenate([z[0, 0][1], z[0, 1][1]], axis=1),
                            jnp.concatenate([z[1, 0][1], z[1, 1][1]], axis=1)], axis=0)

RC = 32
def chunks(): return [slice(o, o + RC) for o in range(0, M, RC)]
def accum(a, x): return x if a is None else a + x
def colsum(x): return jnp.sum(x, axis=0, keepdims=True)

def w_combos(src, dst):
    blk = {(i, j): src[slice(64 * i, 64 * i + 64), slice(256 * j, 256 * j + 256)].astype(f32) for i, j in IJ}
    dst[...] = jnp.concatenate([combo(SU[r], blk) for r in range(7)], axis=0)

def tile_id(t, j): return j * (j + 1) // 2 + t
def p_id(r, a, b):
    if len(SV[r]) == 1:
        _, i, j = SV[r][0]
        return tile_id(2 * a + i, 2 * b + j)
    return 136 + 5 * (b * (b - 1) // 2) + (0, None, 1, 2, None, 3, 4)[r] * b + a
def p_diag(b, i, j): return tile_id(2 * b + i, 2 * b + j)
def d_id(r, a, b): return 24 + 7 * (b * (b - 1) // 2) + r * b + a
def d_diag(b, i, j): return 3 * b + i + j

ORD9 = ("K0 K1 K2 K3 Q3 V0 A3 V1 V2 V3 Q2 Xa3:V1:Q2 O3 O2 Q1 O1 Q0 O0 Xb3:O3:O0 A2 B3 Xa2:B3:B3 A1 C3 EV3 A0 D3 "
        "Xb2:EV3+200:D3 Xa1:EV3+200:D3 EK3 B2 EV2 Xb1:B2:EV2 Xa0:B2:EV2 C2 B1 D2 Xb0:B1+200:D2 C1 EK2 B0 EV1 D1 C0 EK1 D0 EV0 PF0:EK1:EV0 EK0")

OF = ("K0 K1 K2 K3 Q3 V0 A3 V1 V2 V3 Q2 O3 Xa3:V1:O3-300 O2 Q1 O1 Q0 O0 Xb3:O3+330:O0 A2 B3 A1 Xa2:B3:A1-200 C3 EV3 A0 D3 "
      "Xb2:EV3+200:D3 EK3 B2 Xa1:EK3:B2 EV2 C2 Xa0:EV2:EV2")
OF1 = OF + " EK2 D2 Xb1:EK2:D2-300 B1 EV1 Xb0:B1:EV1-400 B0 C1 EV0 PF0:EV0:EV0 D1 C0 EK1 D0 EK0"
OG = ("K0 K1 K2 K3 Q3 V0 A3 V1 V2 V3 Q2 O3 Xa3:V1:O3-300 O2 Q1 O1 Q0 O0 Xb3:O3+330:O0 A2 B3 A1 Xa2:B3:A1-200 C3 EV3 D3 "
      "Xb2:EV3+200:D3 A0 B2 Xa1:A0:B2 EV2 Xa0:EV2:EV2 C2 EK3 D2 EK2 Xb1:EK3+200:EK2-300 B1 EV1 Xb0:B1:EV1-400 B0 C1 EV0 PF0:EV0:EV0 D1 C0 EK1 D0 EK0")
OH = ("K0 K1 K2 K3 Q3 V0 A3 V1 V2 V3 Q2 O3 Xa3:V1:O3-300 O2 Q1 O1 Q0 O0 Xb3:O3+330:O0 A2 B3 A1 Xa2:B3:A1-200 C3 EV3 A0 D3 "
      "Xb2:EV3+200:D3 EK3 B2 EV2 Xa1:EK3:B2-300 Xb1:B2+950:EV2 Xa0:EV2:EV2 C2 B1 D2 Xb0:B1+200:D2 C1 EK2 B0 EV1 D1 C0 EK1 D0 EV0 PF0:EK1:EV0 EK0")
OJ = ("K0 K1 K2 K3 Q3 V0 A3 V1 V2 V3 Q2 O3 Xa3:V1:O3-300 O2 Q1 O1 Q0 O0 Xb3:O3+330:O0 A2 B3 A1 Xa2:B3:A1-200 C3 EV3 D3 "
      "Xb2:EV3+200:D3 A0 B2 Xa1:A0:B2 EV2 Xa0:EV2:EV2 C2 EK3 D2 EK2 Xb1:EK3+200:EK2-300 B1 EV1 Xb0:B1:EV1-400 B0 C1 EV0 ")
OJ1 = OJ + "PF0:EV0:EV0 D1 C0 EK1 D0 EK0 RT0:B1:EV1 MO0:EV0+200:EK0-400"
OJ2 = OJ + "PF0:B1:EV1 D1 C0 EK1 D0 EK0 RT0:EV0:D1 MO0:EV0+200:EK0-400"
OJ3 = OJ + "PF0:EV0:EV0 D1 C0 EK1 D0 EK0 RT0:A3:A3 MO0:B1:EK0-400"
OJ4 = OJ + "PF0:EV0:EV0 D1 C0 EK1 D0 EK0 RT0:EK1:EK0-400 MO0:A2:EK0-400"
OK1 = ("K0 K1 K2 K3 Q3 V0 A3 V1 V2 V3 Q2 O3 Xa3:V1+166:O3-500 O2 Q1 O1 Q0 O0 Xb3:O3+121:O0-166 A2 RT0:O0+500:A2-100 B3 A1 Xa2:B3+34:A1-0 "
       "C3 EV3 D3 Xb2:EV3+186:D3-64 A0 B2 Xa1:A0+134:B2-0 EV2 Xa0:EV2+0:EV2-0 C2 EK3 D2 EK2 Xb1:EK3+201:EK2-500 B1 EV1 Xb0:B1+83:EV1-561 "
       "B0 C1 EV0 PF0:EV0+55:EV0-0 D1 C0 EK1 D0 EK0 MO0:B1+2209:EK0-300")
TAIL = " C1 EK2 B0 EV1 D1 C0 EK1 D0 EV0 PF0:EK1:EV0 EK0"
OA = ("K0 K1 K2 K3 Q3 V0 A3 V1 V2 V3 Q2 O3 Xa3:V1:O3 O2 Q1 O1 Q0 O0 Xb3:O2:O0 A2 B3 A1 Xa2:B3:A1 C3 EV3 A0 D3 "
      "Xb2:EV3+200:D3 EK3 B2 EV2 Xa1:B2:EV2 C2 D2 EK2 Xb1:D2:EK2-300 Xa0:D2:EK2 B1 EV1 Xb0:B1:EV1 C1 B0 D1 C0 EK1 D0 EV0 PF0:EK1:EV0 EK0")
OB = ("K0 K1 K2 K3 Q3 Q2 A3 A2 V0 V1 Xa3:A2:V1 V2 V3 O3 O2 Q1 O1 Q0 O0 Xb3:V2:O0 Xa2:V2:O0 A1 B3 EV3 A0 Xb2:B3:EV3 C3 B2 Xa1:B2:B2 D3 EK3 EV2 "
      "Xb1:D3:EV2 Xa0:D3:EV2 C2 B1 D2 Xb0:B1+200:D2" + TAIL)
OC = ("K0 K1 K2 K3 Q3 Q2 A3 A2 V0 V1 V2 Xa3:A2:V2 V3 O3 O2 Q1 O1 Q0 O0 Xb3:V3:O0 A1 A0 B3 Xa2:A1:B3 EV3 C3 D3 EK3 Xb2:D3:EK3-250 B2 EV2 Xa1:B2:EV2 "
      "C2 D2 EK2 Xb1:D2:EK2-300 Xa0:D2:EK2 B1 EV1 Xb0:B1:EV1 C1 B0 D1 C0 EK1 D0 EV0 PF0:EK1:EV0 EK0")
OD = ("K0 K1 K2 K3 Q3 Q2 A3 A2 V0 V1 V2 Xa3:A2:V2 V3 O3 O2 Q1 O1 Q0 Xb3:V3:Q0 A1 B3 Xa2:A1:B3 A0 EV3 C3 O0 D3 EK3 Xb2:O0:EK3-250 B2 EV2 Xa1:B2:EV2 "
      "C2 D2 EK2 Xb1:D2:EK2-300 Xa0:D2:EK2 B1 EV1 Xb0:B1:EV1 C1 B0 D1 C0 EK1 D0 EV0 PF0:EK1:EV0 EK0")
OE = ("K0 K1 K2 K3 Q3 Q2 A3 A2 V0 V1 V2 Xa3:A2:V2 V3 O3 O2 Q1 O1 Q0 Xb3:V3:Q0 A1 B3 Xa2:A1:B3 A0 EV3 C3 O0 D3 EK3 Xb2:O0:EK3-250 B2 EV2 Xa1:B2:EV2 "
      "Xa0:B2:EV2 C2 EK2 D2 Xb1:EK2:D2-300 B1 EV1 Xb0:B1:EV1 C1 B0 D1 C0 EK1 D0 EV0 PF0:EK1:EV0 EK0")


class NS:
    def __init__(self, d):
        self._d = d
    def __getattr__(self, n):
        return self._d[n]


class Sched:
    def __init__(self, h):
        self.load, self.toks = [0, 0, 0, 0], []
        self.never = lax.broadcasted_iota(i32, (8, T), 0) + h < 0
    def now(self): return sum(self.load) // 4
    def _track(self, x, k):
        for c in range(-(-x.shape[1] // T)):
            t0 = 0
            for _ in range(-(-k // T)):
                q = self.load.index(min(self.load))
                t0 = max(t0, self.load[q])
                self.load[q] += x.shape[0]
            if x.shape[0] > CP:
                self.toks.extend((t0 + 8 * i, x, i, c) for i in range(x.shape[0] // 8))
        return x
    def nn(self, a, b): return self._track(nn(a, b), a.shape[1])
    def nt(self, a, b): return self._track(nt(a, b), a.shape[1])
    def gate(self, t0, t1, n):
        it = iter(range(n))
        def stamps(k):
            out = []
            for _ in range(k):
                t = t0 + (t1 - t0) * next(it) / n
                _, x, i, c = min(self.toks, key=lambda e: abs(e[0] - t))
                out.append(x[8 * i:8 * i + 8, c * T:(c + 1) * T])
            return cat(out, 0).reshape(k, 8, T)
        return stamps
    def tie(self, stamp, x):
        return jnp.where(self.never[None], stamp, x[None])
    def hold(self, stamp, x):
        k = stamp.shape[0]
        if x.dtype != f32: stamp = pltpu.bitcast(stamp, x.dtype)
        return jnp.where(self.never[None, None], stamp[:, None], x.reshape(k, -1, 8, T)).reshape(x.shape)


def make(cfg):
    names = list(SCR)
    scr_shapes = {n: (V(v.shape[:-1] + (v.shape[-1] + T,), v.dtype) if n in cfg.get("pad", "").split() else v) for n, v in SCR.items()}
    scope = jax.named_scope if cfg.get('scopes') else (lambda n: contextlib.nullcontext())

    def kernel(xT_h, c_h, goT_h, wq_h, wuk_h, wuv_h, woT_h, wr_ref, wg_h, wu_h, wdT_h,
               outT_h, dxT_h, dc_h, dwq_h, dwuk_h, dwuv_h, dwoT_h, dwr_ref, dwg_h, dwu_h, dwdT_h, *scr):
        raw = dict(zip(names, scr))
        s = NS({**{n: Pk(raw[n]) if n in PACKED else raw[n] for n in names},
                **{n: Pk(raw[v[0]], *v[1:]) for n, v in VIEWS.items()}})
        sem = s.sem
        w_h = (wq_h, wuk_h, wuv_h); dw_h = (dwq_h, dwuk_h, dwuv_h)
        m_h = (wg_h, wu_h, wdT_h); dm_h = (dwg_h, dwu_h, dwdT_h)
        cp = pltpu.make_async_copy
        XW = 512; NX = S // XW
        def ch(b, w=XW): return pl.ds(pl.multiple_of(b * w, w), w)
        def tile(b): return ch(b, T)

        def wait_all(buf, q): cp(buf, buf, sem.at[q]).wait()
        SX, SG, SC = 7, 15, 19
        def w_start(w, p, out):
            n = WROWS[w] // 4
            for e in range(4):
                far = (dw_h if out else w_h)[w].at[:, e, p]
                near = (s.wout if out else s.wi).at[WOFF[w]:WOFF[w] + n, 2 * e:2 * e + 2, :]
                (cp(near, far, sem.at[4]) if out else cp(far, near, sem.at[0])).start()
        def wk_start(t):
            for e in range(4):
                far = wuk_h.at[:, e, jnp.minimum(t, H - 1) >> 1]
                cp(far, s.wkn.at[0:DC // 4, 2 * e:2 * e + 2, :], sem.at[1]).start()
        def wk_wait(): wait_all(s.wkn.at[0:DC // 4], 1)
        def wo_in(t): return cp(woT_h.at[jnp.minimum(t, H - 1)], s.woi, sem.at[5])
        def wo_out(p): return cp(s.woo, dwoT_h.at[pl.ds(2 * p, 2)], sem.at[6])
        def m_start(p, out):
            for w in range(3):
                for t in range(FT):
                    far = (dm_h if out else m_h)[w].at[:, tile(p * FT + t)]
                    (cp(s.mo.at[w * FT + t], far, sem.at[3]) if out else cp(far, s.mi.at[w * FT + t], sem.at[2])).start()
        def w_load(w, h):
            x = s.wkn[0:DC // 4] if w == 3 else s.wi[WOFF[w]:WOFF[w] + WROWS[w] // 4]
            x = pltpu.bitcast(x.reshape(x.shape[0] * 8, D), u32)
            sh = jnp.asarray(16 * (1 - (h & 1)), i32).astype(u32)
            return pltpu.bitcast((x << sh) & jnp.uint32(0xFFFF0000), f32)

        cp(wr_ref, s.wr1, sem.at[23]).start()
        @pl.loop(0, NB)
        def _(n):
            cp(xT_h.at[:, tile(n)], s.st_x.at[n], sem.at[SX + (n >> 1)]).start()
        wk_start(0)
        @pl.loop(0, NB)
        def _(n):
            cp(goT_h.at[:, tile(n)], s.st_go.at[n], sem.at[SG + (n >> 2)]).start()
        @pl.loop(0, NB)
        def _(n):
            cp(c_h.at[ch(n >> 2), tile(n & 3)], s.st_c.at[n & 3, ch(n >> 2)], sem.at[SC + (n >> 2)]).start()
        for w in range(3): w_start(w, 0, False)
        wo_in(0).start()

        for a in (s.y, s.gosel, s.dxsel, s.zero, s.stat, s.upd, s.mr): a[...] = jnp.zeros_like(a)
        @pl.loop(0, 2)
        def _(n):
            for nm in PIN:
                raw[nm][pl.ds(pl.multiple_of(n * 8, 8), 8), 0:128] = jnp.zeros((8, 128), raw[nm].dtype)
        cp(wr_ref, s.wr1, sem.at[23]).wait()
        s.wr[0:1, :] = s.wr1[...].astype(f32).reshape(1, M)
        s.wrb[...] = jnp.broadcast_to(s.wr[0:1, :], (T, M)).T

        def combos(src, ck):
            arr = (s.goT, s.xnT, s.cT)[src].ref
            if ck is None:
                zv, st_, hv = arr.at[256:288], 8, raw["hz"].at[src * (7 * MQ) + 64:(src + 1) * (7 * MQ)]
            else:
                o = pl.multiple_of(8 * ck, 8)
                zv, st_ = arr.at[pl.ds(o, 200)], 64
                bv = raw["bs"].at[pl.ds(pl.multiple_of(src * 640 + o, 8), 584)]
                hv = raw["hz"].at[pl.ds(pl.multiple_of(src * (7 * MQ) + o, 8), 13 * (MQ // 2) + 8)]
            for q in range(4):
                z = {(i, j): up(zv[st_ * i:st_ * i + 8, sl(4 * q + j, 4 * q + j + 1)]).astype(f32) for i in range(4) for j in range(4)}
                out = [(z[0, j] + z[1, j]) + (z[2, j] + z[3, j]) for j in range(4)]
                for i in range(4):
                    a, b, c_ = (j for j in range(4) if j != i)
                    out.append((z[i, i] - z[i, a]) - (z[i, b] + z[i, c_]))
                out += [z[i, j] + z[j, i] for i, j in HP]
                for k, y in enumerate(out):
                    hv[k * (MQ // 2):k * (MQ // 2) + 8, sl(q, q + 1)] = pk(y)
                if ck is None: continue
                for i0, j0 in IJ:
                    blk = {(i, j): z[i0 + 2 * i, 2 * j0 + j] for i, j in IJ}
                    for k, r in enumerate(R2):
                        bv[128 * k + 64 * i0:128 * k + 64 * i0 + 8, sl(2 * q + j0, 2 * q + j0 + 1)] = pk(combo(SV[r], blk))

        with scope("ln"):
            @pl.loop(0, NB + 1)
            def _(n):
                @pl.when(jnp.logical_and((n & 1) == 0, n < NB))
                def _():
                    wait_all(s.st_x.at[pl.ds(n, 2)], SX + (n >> 1))
                m, n1 = jnp.maximum(n - 1, 0), jnp.minimum(n, NB - 1)
                cs, cn = tile(m), tile(n1)
                mu, sd = s.stat[0:1, cs], s.stat[1:2, cs]
                x0 = s.st_x[n1, 0:16, :].astype(f32)[0:1]
                ar = a1 = a2 = None
                for rr in chunks():
                    x = s.st_x[m, rr, :].astype(f32)
                    s.xnT[rr, cs] = rb(x - mu) / sd
                    xn = s.xnT[rr, cs].astype(f32)
                    s.acc[0, rr, cs] = x + xn
                    ar = accum(ar, xn * s.wrb[rr])
                    d = s.st_x[n1, rr, :].astype(f32) - x0
                    a1 = accum(a1, d); a2 = accum(a2, d * d)
                s.r[pl.ds(m, 1), :] = rb(colsum(ar))
                e1 = colsum(a1) / M
                var = jnp.maximum(colsum(a2) / M - e1 * e1, 0.0)
                s.stat[0:1, cn] = rb(x0 + e1)
                s.stat[1:2, cn] = rb(jnp.sqrt(rb(rb(var) + EPS_B)))

        col = (lax.broadcasted_iota(i32, (NB, T), 0) * T + lax.broadcasted_iota(i32, (NB, T), 1)).astype(f32)
        row = lax.broadcasted_iota(i32, (CP, T), 0)
        lane = lax.broadcasted_iota(i32, (CP, T), 1)
        def pick(r):
            mx = jnp.max(jnp.max(r, axis=0, keepdims=True), axis=1, keepdims=True)
            ix = jnp.min(jnp.min(jnp.where(r == mx, col, float(S)), axis=0, keepdims=True), axis=1, keepdims=True)
            return jnp.where(col == ix, -jnp.inf, r), jnp.broadcast_to(mx, (8, T)), ix.astype(i32)[0, 0]
        def gather(arr, n, tok):
            x = arr[al, tile(tok >> 7)]
            l = tok & (T - 1)
            e = jnp.where(lax.broadcasted_iota(i32, (T, T), 0) == l, 1.0, 0.0).astype(bf16)
            e1 = jnp.where(jnp.logical_and(row == n, lane == l), 1.0, 0.0).astype(bf16)
            return nn(x, e), nt(e1, x)

        def after(n, x, *bufs):
            o = pl.ds(pl.multiple_of((n & 1) * 8, 8), 8)
            t = None
            for b in bufs:
                y = b[o, 0:T] if len(b.shape) == 2 else b[1, o, 0:T]
                y = y if y.dtype == u32 else pltpu.bitcast(y, u32)
                t = y if t is None else t | y
            never = lax.broadcasted_iota(i32, (8, T), 0) + n < 0
            k = cfg.get("tk", 0) * 8
            return jnp.concatenate([x[:k]] * (k > 0) + [jnp.where(never, pltpu.bitcast(t, f32), x[k:k + 8]), x[k + 8:]], axis=0)

        def route(n, carry):
            r, mx, tok, rsel = carry
            @pl.when((n & 1) == 0)
            def _():
                wait_all(s.st_go.at[pl.ds(2 * n, 4)], SG + (n >> 1))
            nxt = pick(r)
            rsel = jnp.where(row == n, sigmoid_b(mx)[0:1], rsel)
            tok = jnp.clip(tok, 0, S - 1)
            s.tok[n] = tok
            xb, xr = gather(s.xnT, n, tok)
            combos(1, n)
            for j in range(2):
                for rr in chunks():
                    go = s.st_go[2 * n + j, rr, :]
                    s.goT[rr, tile(2 * n + j)] = go
            s.xb[0, n] = after(n, xb, raw["bs"], raw["hz"], raw["goT"])
            s.y[...] += xr
            return nxt + (rsel,)
        with scope("route"):
            wk_wait()
            init = pick(s.r[...]) + (jnp.zeros((CP, T), f32),)
            s.wkT[...] = w_load(3, 0).astype(bf16).T
            combos(1, None)
            w_combos(s.wkT, s.uk)
            s.rs[...] = lax.fori_loop(0, C, route, init)[3]
            s.xsel[...] = s.y[...].astype(bf16)
            s.y[...] = jnp.zeros_like(s.y)
            combos(0, None)

        with scope("latent"):
            @pl.loop(0, C)
            def _(n):
                @pl.when((n & 1) == 0)
                def _():
                    wait_all(s.st_c.at[:, ch(n >> 1)], SC + (n >> 1))
                gb, gr = gather(s.goT, n, jnp.clip(s.tok[n], 0, S - 1))
                ct = [s.st_c[i, ch(n, 2 * T), :].T for i in range(4)]
                combos(0, n)
                if cfg.get("init1", 1):
                    for j in range(2):
                        for rr in chunks(): s.acc[1, rr, tile(2 * n + j)] = s.st_go[2 * n + j, rr, :].astype(f32)
                s.xb[1, n] = rb(after(n, gb, raw["bs"], raw["hz"], s.acc) * s.rs[pl.ds(n, 1), :])
                s.gosel[...] += gr
                for i in range(4): s.cT[sl(i, i + 1), ch(n, 2 * T)] = ct[i]
            s.dy[...] = (s.gosel[...] * s.rs[:, 0:1]).astype(bf16)
        with scope("combos"):
            @pl.loop(0, 8)
            def _(n):
                combos(2, n)

        def main_step(h):
            odd = (h & 1) == 1
            even = (h & 1) == 0
            p = h >> 1
            wo_in(h).wait()
            @pl.when(even)
            def _():
                wait_all(s.wi, 0)
            @pl.when(h >= 1)
            def _():
                wk_wait()
            @pl.when(jnp.logical_and(even, jnp.logical_and(p >= 2, p <= NFC + 1)))
            def _():
                wait_all(s.mo, 3)
            def anchor(buf, x):
                buf[pl.ds(buf.shape[0] - 2 + (h & 1), 1), 0:8] = x.astype(bf16)
            def pull(buf):
                return buf[pl.ds(buf.shape[0] - 2 + (h & 1), 1), 0:8][0].astype(f32)
            def starts(k):
                if k == 0:
                    @pl.when(jnp.logical_and(even, p < NFC))
                    def _():
                        m_start(p, False)
                    return pull(s.mi)
                @pl.when(odd)
                def _():
                    for w in range(3): w_start(w, jnp.minimum(p + 1, H // 2 - 1), False)
                wo_in(h + 1).start()
                wk_start(h + 2)
                return pull(s.wkn)
            with scope('headA'):
                if cfg.get("skipA"):
                    for a_ in (s.em, s.ec, s.wm, s.wc): a_[h & 1, h & 1, 0:8, 0:128] = s.mr[0:8] + starts(0) + starts(1) + s.y[0:8, 0:128] + s.dxsel[0:8, 0:128]
                else:
                    head_body(cfg, s, h, w_load, starts)

            def done(w, x=None):
                if w == "wo": wo_out(p).start()
                elif w == "moe":
                    @pl.when(jnp.logical_and(p >= 1, p <= NFC))
                    def _():
                        m_start(p - 1, True)
                elif w in (0, 1, 2): w_start(w, p, True)
                else:
                    @pl.when(h == H - 1)
                    def _():
                        if w == "out":
                            cp(s.wr1, dwr_ref, sem.at[23]).start()
                            for n in range(NB): cp(s.st_x.at[n], outT_h.at[:, sl(n, n + 1)], sem.at[SX]).start()
                        else:
                            for i in range(4): cp(s.st_c.at[i], dc_h.at[:, sl(i, i + 1)], sem.at[SC]).start()
                if x is not None: anchor(s.wout, x)
            @pl.when(odd)
            def _():
                @pl.when(p < NFC)
                def _():
                    wait_all(s.mi.at[0:3 * FT], 2)
                @pl.when(p >= 1)
                def _():
                    wo_out(p - 1).wait()
                    wait_all(s.wout.at[0:WS], 4)
                with scope('pairP'):
                    if cfg.get("skipP"):
                        for a_ in (s.em, s.ec): s.dcT[0:8, 0:128] += a_[h & 1, h & 1, 0:8, 0:128]
                        for a_ in (s.wm, s.wc): s.dcT[0:8, 0:128] += a_[h & 1, h & 1, 0:8, 0:128]
                    else:
                        pair_body(cfg, s, h, done)

        with scope('main'):
            pl.loop(0, H)(main_step)

        def fin(n, carry):
            m = jnp.maximum(n - 1, 0)
            cs, cn = tile(m), tile(jnp.minimum(n, NB - 1))
            m1, m2, rstd = carry[0][0:1], carry[1][0:1], 1.0 / s.stat[1:2, cs]
            a1 = a2 = None
            for rr in chunks():
                go = s.goT[rr, cs].astype(f32)
                d = s.acc[1, rr, cs] if cfg.get("init1", 1) else s.acc[1, rr, cs] + go
                s.st_go[m, rr, :] = (go + (d - m1 - s.xnT[rr, cs].astype(f32) * m2) * rstd).astype(bf16)
                dxn = s.acc[1, rr, cn] if cfg.get("init1", 1) else s.acc[1, rr, cn] + s.goT[rr, cn].astype(f32)
                a1 = accum(a1, dxn); a2 = accum(a2, dxn * s.xnT[rr, cn].astype(f32))
            @pl.when(n >= 1)
            def _():
                cp(s.st_go.at[m], dxT_h.at[:, cs], sem.at[SG]).start()
            return tuple(jnp.broadcast_to(colsum(a) / M, (8, T)) for a in (a1, a2))
        with scope("fin"):
            lax.fori_loop(0, NB + 1, fin, (jnp.zeros((8, T), f32), jnp.zeros((8, T), f32)))
        wo_in(H).wait(); wk_wait(); wait_all(s.wi, 0)
        wo_out(H // 2 - 1).wait()
        wait_all(s.wout.at[0:WS], 4)
        cp(s.wr1, dwr_ref, sem.at[23]).wait(); wait_all(s.st_c, SC); wait_all(s.st_x, SX); wait_all(s.st_go, SG)

    def fn(A_x, A_c_kv, A_w_q, A_w_uk, A_w_uv, A_w_o, B_x, B_w_r, B_w_gate, B_w_up, B_w_down, grad_out):
        xT = A_x.reshape(S, M).T; goT = grad_out.reshape(S, M).T; c = A_c_kv.reshape(S, DC)
        woT = jnp.swapaxes(A_w_o, 1, 2)
        wdT = B_w_down.T
        sds = jax.ShapeDtypeStruct
        hbm = pl.BlockSpec(memory_space=pl.ANY)
        vm = pl.BlockSpec(memory_space=pltpu.VMEM)
        outs = pl.pallas_call(
            kernel,
            in_specs=[hbm] * 11,
            out_specs=[hbm] * 11,
            out_shape=[sds((M, S), bf16), sds((M, S), bf16), sds((S, DC), bf16), sds((M // 4, 4, H // 2, 2, D), bf16),
                       sds((DC // 4, 4, H // 2, 2, D), bf16), sds((DC // 4, 4, H // 2, 2, D), bf16), sds((H, M, D), bf16), sds((M,), bf16),
                       sds((M, F), bf16), sds((M, F), bf16), sds((M, F), bf16)],
            scratch_shapes=list(scr_shapes.values()),
            compiler_params=pltpu.CompilerParams(vmem_limit_bytes=124 * 1024 * 1024,
                                                 disable_bounds_checks=bool(cfg.get("nobc"))),
            name="mla",
        )(xT, c, goT, A_w_q.reshape(M // 4, 4, H // 2, 2, D), A_w_uk.reshape(DC // 4, 4, H // 2, 2, D), A_w_uv.reshape(DC // 4, 4, H // 2, 2, D), woT, B_w_r, B_w_gate, B_w_up, wdT)
        outT, dxT, dc, dwq, dwuk, dwuv, dwoT, dwr, dwg, dwu, dwdT = outs
        return (outT.T.reshape(1, S, M), dxT.T.reshape(1, S, M), dc.reshape(1, S, DC),
                dwq.reshape(M, H, D), dwuk.reshape(DC, H, D), dwuv.reshape(DC, H, D),
                jnp.swapaxes(dwoT, 1, 2), dwr, dwg, dwu, dwdT.T)
    return fn


def head_body(cfg, s, h, w_load, starts):
    tri = lax.broadcasted_iota(i32, (T, T), 0) <= lax.broadcasted_iota(i32, (T, T), 1)
    sc = Sched(h)
    nn, nt = sc.nn, sc.nt
    st = {}
    order = cfg.get("order", OK1)
    hs = h & 1
    span = {}
    def const(c):
        if "pull" not in st: return c
        return jnp.where(sc.never, st.pop("pull"), c)[0:1, 0:1] if cfg.get("c11") else jnp.tile(jnp.where(sc.never, st.pop("pull"), c)[0:1], (1, 2))
    def gate(a, b, n):
        a, _, sk = a.partition("+"); b, _, tl = b.partition("-")
        return sc.gate(span[a][0] + int(sk or cfg.get("skip", 64)), span[b][1] - int(tl or cfg.get("tail", 64)), n)

    def W():
        wq = w_load(0, h); s.wm[1, hs] = wq
        s.wqT[al, :M] = wq.astype(bf16).T
        wv = w_load(2, h); s.wc[0, hs] = wv
        s.wvT[...] = wv.astype(bf16).T
        s.wo[al, :M] = s.woi[...].T
        w_combos(s.wo, s.uo); w_combos(s.wvT, s.uv); w_combos(s.wqT, s.uq)
    def fwd(u, b, init=None):
        return join(scatter(SW, {r: nn(u[slice(64 * r, 64 * r + 64), al], b(r)) for r in cfg.get("fo", range(7))}, init))
    def bs(src, n):
        def get(r):
            if r not in R2:
                _, i, j = SV[r][0]
                return (s.goT, s.xnT, s.cT)[src][slice(i * CH, (i + 1) * CH), sl(2 * n + j, 2 * n + j + 1)]
            k = src * 5 + R2.index(r)
            return s.bs[slice(k * CH, (k + 1) * CH), sl(n, n + 1)]
        return get
    def put(z, n, xT, xc, table, on):
        xT[al, sl(2 * n, 2 * n + 2)] = z
        if on:
            blk = {(i, j): z[64 * i:64 * i + 64, j * T:(j + 1) * T] for i, j in IJ}
            xc[al, sl(n, n + 1)] = jnp.concatenate([combo(table[r], blk) for r in range(7)], axis=0)
    def K(J):
        if cfg.get("sK", 1):
            for n in range(2 * J, 2 * J + 2):
                put(fwd(s.uk, bs(2, n)), n, s.kT, s.kc, SU, n < NP - 1)
        else:
            z = nn(s.wkT[...], s.cT[al, sl(4 * J, 4 * J + 4)])
            for n in range(2 * J, 2 * J + 2):
                put(z[:, sl(2 * n - 4 * J, 2 * n - 4 * J + 2)], n, s.kT, s.kc, SU, n < NP - 1)
        s.k[sl(4 * J, 4 * J + 4), al] = s.kT[al, sl(4 * J, 4 * J + 4)].T
    def Q(J):
        if cfg.get("sQ", 1):
            for n in range(2 * J, 2 * J + 2):
                hi = nn(s.wqT[al, 512:M], s.xnT[512:M, sl(2 * n, 2 * n + 2)])
                put(fwd(s.uq, bs(1, n), hi) * const(QSCALE), n, s.qT, s.qc, SW, n > 0)
            return
        z = nn(s.wqT[al, :M], s.xnT[al, sl(4 * J, 4 * J + 4)]) * QSCALE
        for n in range(2 * J, 2 * J + 2):
            put(z[:, sl(2 * n - 4 * J, 2 * n - 4 * J + 2)], n, s.qT, s.qc, SW, n > 0)
    def Vv(J):
        for n in range(2 * J, 2 * J + 2):
            put(fwd(s.uv, bs(2, n)), n, s.vT, s.vc, SU, n < NP - 1)
            x = [pltpu.bitcast(s.vT[al, sl(2 * n + j, 2 * n + j + 1)].T, u32).reshape(8, 1, 8, T) for j in range(2)]
            s.kv[n * T:(n + 1) * T, T:] = jnp.concatenate(x, axis=1).reshape(T, T)
    def O(J):
        for n in range(2 * J, 2 * J + 2):
            hi = nn(s.wo[al, 512:M], s.goT[512:M, sl(2 * n, 2 * n + 2)])
            put(fwd(s.uo, bs(0, n), hi), n, s.oT, s.oc, SW, n > 0)
    def col(j, t0=0, t1=None): return sl(tile_id(t0, j), tile_id(j if t1 is None else t1 - 1, j) + 1)
    def col8(j): return slice(tile_id(0, j) * 8, tile_id(j, j) * 8 + 8)
    def A(J):
        for j in range(4 * J + 3, 4 * J - 1, -1):
            x = nn(s.k[sl(0, j + 1), al], s.qT[al, sl(j, j + 1)])
            sd = jnp.where(tri, x[j * T:, :], -1e9)
            x = sd if j == 0 else jnp.concatenate([x[:j * T, :], sd], axis=0)
            s.ml[col8(j), :T] = jnp.max(x.reshape(j + 1, 16, 8, T), axis=1).reshape((j + 1) * 8, T)
            st["m", j] = jnp.broadcast_to(jnp.max(s.ml[col8(j), :T], axis=0, keepdims=True), (8, T))
            s.sT[col(j), :] = x
    def Xa(J, wa, wb):
        ga = cfg.get("GA", 4)
        stamps = gate(wa, wb, (16 * J + 10) * ga)
        for j in range(4 * J, 4 * J + 4):
            m = st["m", j]
            k = (j + 1) * ga
            p = jnp.exp2(s.sT[col(j), :].reshape(k, 16 // ga, 8, T) - sc.tie(stamps(k), m)[:, None])
            s.ml[col8(j), T:] = jnp.sum(p.reshape(j + 1, 16, 8, T), axis=1).reshape((j + 1) * 8, T)
            st["c", j] = m + jnp.log2(jnp.sum(s.ml[col8(j), T:], axis=0, keepdims=True))
    def Xb(J, wa, wb):
        stamps = gate(wa, wb, (16 * J + 10) * 2)
        for b in (2 * J + 1, 2 * J):
            if b > 0:
                tk = stamps(8 * b)
                blk = {}
                for j in range(2):
                    c = sc.tie(tk, st["c", 2 * b + j]).reshape(b, 1, 8, 1, 8, T)
                    p = jnp.exp2(s.sT[col(2 * b + j, 0, 2 * b), :].reshape(b, 2, 8, 2, 8, T) - c)
                    s.PT[col(2 * b + j, 0, 2 * b), al] = p.reshape(2 * b * T, T)
                    for i in range(2): blk[i, j] = p[:, i].reshape(b * T, T)
                for r in range(7):
                    if len(SV[r]) == 2:
                        s.PT[sl(p_id(r, 0, b), p_id(r, 0, b) + b), al] = combo(SV[r], blk)
            for j in range(2):
                k = 2 * (j + 1)
                c = sc.tie(stamps(k), st["c", 2 * b + j])[:, None]
                s.PT[col(2 * b + j, 2 * b), al] = jnp.exp2(s.sT[col(2 * b + j, 2 * b), :].reshape(k, 8, 8, T) - c).reshape(k * 64, T)
    def tiles(Y, ids, axis):
        if axis == 0 and all(b - a == 1 for a, b in zip(ids, ids[1:])): return Y[sl(ids[0], ids[-1] + 1), al]
        return cat([Y[sl(i, i + 1), al] for i in ids], axis)
    def left(Y, cid, did, xT, xc, b):
        diag = lambda: jnp.concatenate([nn(xT[al, sl(2 * b, 2 * b + j + 1)], tiles(Y, [did(b, i, j) for i in range(j + 1)], 0))
                                        for j in range(2)], axis=1)
        if b == 0: return diag()
        prods = lambda: {r: nn(xc[slice(64 * r, 64 * r + 64), sl(0, b)], tiles(Y, [cid(r, a, b) for a in range(b)], 0))
                         for r in cfg.get("lo", (0, 6, 5, 3, 4, 1, 2))}
        if cfg.get("dl"):
            z = join(scatter(SW, prods()))
            return z + diag()
        z = diag()
        return join(scatter(SW, prods(), z))
    def right(Y, cid, did, xT, xc, a):
        diag = lambda: jnp.concatenate([nt(xT[al, sl(2 * a + i, 2 * a + 2)], tiles(Y, [did(a, i, j) for j in range(i, 2)], 1))
                                        for i in range(2)], axis=1)
        if a == NP - 1: return diag()
        prods = lambda: {r: nt(xc[slice(64 * r, 64 * r + 64), sl(a + 1, NP)],
                               tiles(Y, [cid(r, a, b) for b in range(a + 1, NP)], 1)) for r in cfg.get("ro", range(7))}
        if cfg.get("dl"):
            z = join(scatter(SU, prods()))
            return z + diag()
        z = diag()
        return join(scatter(SU, prods(), z))
    def B(J):
        for b in (2 * J + 1, 2 * J):
            cs = sl(2 * b, 2 * b + 2)
            ctxT = left(s.PT, p_id, p_diag, s.vT, s.vc, b)
            st["dl", b] = jnp.sum(ctxT * s.oT[al, cs].astype(f32), axis=0, keepdims=True)
            s.em[0, hs, :, cs] = ctxT
    def Cc(J):
        dp = {}
        for b in (2 * J + 1, 2 * J):
            if b > 0:
                dp[b] = nn(s.v[sl(0, 2 * b), al], s.oT[al, sl(2 * b, 2 * b + 2)]) - st["dl", b]
        for b in (2 * J + 1, 2 * J):
            vd = s.kv[b * T:(b + 1) * T, T:].reshape(8, 2, 8, T)
            dp[b, 1] = nn(s.v[sl(2 * b, 2 * b + 2), al], s.oT[al, sl(2 * b + 1, 2 * b + 2)]) - st["dl", b][:, T:]
            dp[b, 0] = nn(up(vd[:, 0].reshape(64, T)), s.oT[al, sl(2 * b, 2 * b + 1)]) - st["dl", b][:, :T]
        def deint(x, i): return x.reshape(-1, 2, 16, T)[:, i].reshape(-1, T)
        for b in (2 * J + 1, 2 * J):
            if b > 0:
                blk = {}
                for j in range(2):
                    p = s.PT[col(2 * b + j, 0, 2 * b), al].astype(f32).reshape(b, 2, T, T)
                    for i in range(2):
                        blk[i, j] = p[:, i].reshape(b * T, T) * deint(dp[b][:, j * T:(j + 1) * T], i)
                for r in range(7):
                    s.dST[sl(d_id(r, 0, b), d_id(r, 0, b) + b), al] = combo(SV[r], blk)
            for i, j in ((0, 0), (0, 1), (1, 1)):
                x = dp[b, 0] if j == 0 else deint(dp[b, 1], i)
                s.dST[sl(d_diag(b, i, j), d_diag(b, i, j) + 1), al] = tiles(s.PT, [p_diag(b, i, j)], 0).astype(f32) * x
    def Dd(J):
        for b in (2 * J + 1, 2 * J):
            s.em[1, hs, :, sl(2 * b, 2 * b + 2)] = left(s.dST, d_id, d_diag, s.kT, s.kc, b) * const(SCALE)
    def EV(I):
        for a in (2 * I + 1, 2 * I):
            s.ec[0, hs, :, sl(2 * a, 2 * a + 2)] = right(s.PT, p_id, p_diag, s.oT, s.oc, a)
    def EK(I):
        for a in (2 * I + 1, 2 * I):
            s.ec[1, hs, :, sl(2 * a, 2 * a + 2)] = right(s.dST, d_id, d_diag, s.qT, s.qc, a) * LN2
    def PF(_, wa, wb):
        stamps = gate(wa, wb, 8 + 8 + 9 + 4)
        x = pk(sc.hold(stamps(8), w_load(3, h + 1)).astype(bf16).T)
        s.wc[1, hs] = sc.hold(stamps(8), w_load(1, h))
        s.wm[0, hs] = sc.hold(stamps(9), s.woi[...].astype(f32))
        st["pull"] = starts(1)
        tk = stamps(4)
        for c in range(DC // T):
            y = x[:, c * T:(c + 1) * T]
            s.wkT.ref[:, c * T:(c + 1) * T] = jnp.concatenate([sc.hold(tk, y[:32]), sc.hold(tk, y[32:])], axis=0)
        w_combos(s.wkT, s.uk)
    def MO(_, wa, wb):
        RG = cfg.get("RG", 36)
        stamps = gate(wa, wb, 5 * RG)
        for src, job in ((0, FT * hs), (0, FT * hs + 1), (0, FT * hs + 2), (1, 2 * FT + hs), (1, 2 * FT + 1 + hs)):
            r = s.mr[pl.ds(pl.multiple_of(job * C, C), C), :]
            o = sc.hold(stamps(RG), s.xb[src, 0]) * r[0:1]
            for c in range(1, C):
                o = o + s.xb[src, c] * r[c:c + 1]
            s.mo[job] = o.astype(bf16)
    def RT(_, wa, wb):
        stamps = gate(wa, wb, 40)
        rs = sc.hold(stamps(2), s.rs[...])[:, 0:1]
        y = rb(s.y[...])
        dr = rb(rb(jnp.sum(rb(s.gosel[...] * y), axis=1, keepdims=True)) * rb(rs * (1.0 - rs)))
        s.wr1[...] = jnp.sum(dr * s.xsel[...].astype(f32), axis=0).astype(bf16)
        s.upd[:CP, :M] = rb(y * rs)
        s.upd[CP:, :M] = s.dxsel[...] + dr * s.wr[0:1, :]
        c = jnp.maximum(h - (H - C), 0)
        tok = jnp.clip(s.tok[c], 0, S - 1)
        hit = lax.broadcasted_iota(i32, (M, T), 1) == jnp.where(h < H - C, -1, tok & (T - 1))
        cs = pl.ds(pl.multiple_of((tok >> 7) * T, T), T)
        stamps(8)
        vb = []
        for k in range(2):
            v = jnp.broadcast_to(s.upd[pl.ds(k * CP + c, 1), :], (8, 5 * T))
            v = jnp.concatenate([sc.hold(stamps(1), v[:, sl(t, t + 1)]) for t in range(5)], axis=1)
            vb.append(jnp.broadcast_to(v[0:1], (T, 5 * T)).T[:M])
        stamps(2)
        for k in range(2):
            s.acc[k, :, cs] = sc.hold(stamps(9), s.acc[k, :, cs]) + jnp.where(hit, vb[k], 0.0)
    ops = dict(MO=MO, RT=RT, K=K, V=Vv, Q=Q, O=O, A=A, Xa=Xa, Xb=Xb, B=B, C=Cc, D=Dd, EV=EV, EK=EK, PF=PF)
    st["pull"] = starts(0)
    W()
    for tk_ in order.split():
        name, *win = tk_.split(":")
        assert name not in span
        t0 = sc.now()
        ops[name[:-1]](int(name[-1]), *win)
        span[name] = (t0, sc.now())
    assert len(span) == 4 * len(ops) - 9, len(span)


def pair_body(cfg, s, h, done):
    sc = Sched(h)
    nn, nt = sc.nn, sc.nt
    first = h == 1
    fill = []
    def filler():
        if fill: fill.pop(0)()

    class Phase:
        def __init__(self, kind, side):
            self.kind, self.side = kind, side
            self.R = MQ if side else T
            self.e, self.w = (s.em, s.wm) if side else (s.ec, s.wc)
            self.src = kind if side else 2
            self.z = (s.goT, s.xnT, s.cT)[self.src]
            self.buf = (s.PT, s.dST)[side]
            self.ubuf = (s.dST, s.PT)[side]
            self.tmp0 = kind * 36 * MQ
            self.wix = (3, 0)[kind] if side else (2, 1)[kind]
        def parts(self, i):
            return [(i * T, T)] + ([(DC + 16 * i, 16)] if self.side else [])
        def quarter(self, get, i): return cat([get(slice(o, o + n)) for o, n in self.parts(i)], 0)
        def wid(self, r, q): return self.kind * 104 + 4 * r + q
        def urows(self, r):
            o = (208 + 30 * self.kind) * T + r * MQ
            return slice(o, o + self.R)
        def tmp(self, k): return slice(self.tmp0 + k * MQ, self.tmp0 + k * MQ + self.R)
        def b(self, j, k):
            return jnp.concatenate([self.e[self.kind, k, :, sl(4 * q + j, 4 * q + j + 1)] for q in range(4)], axis=0)
        def put_w(self, r, x): self.buf[sl(self.wid(r, 0), self.wid(r, 0) + 4), al] = x
        def times(self, tk, c, x):
            return (sc.tie(tk, jnp.full((8, T), c, f32))[:, None] * x.reshape(tk.shape[0], -1, 8, T)).reshape(x.shape)
        def prep_diag(self, t0=None, t1=None):
            stamps = None if t0 is None else sc.gate(t0, t1, 4 * NGP)
            for j in range(4):
                b0 = self.b(j, 0)
                if stamps is not None: b0 = sc.hold(stamps(NGP), b0)
                self.put_w(j, b0)
                self.put_w(4 + j, self.b(j, 1) - HT[j] * b0)
        def prep_pair(self, k, stamps):
            i, j = HP[k]
            bi0, bj0 = self.b(i, 0), self.b(j, 0)
            n_ij = (self.b(i, 1) + self.b(j, 1)) - self.times(stamps(NGP), HT[i], bi0 + bj0)
            c = n_ij + (HT[i] - HT[j]) * bj0
            self.put_w(9 + 3 * k, n_ij)
            self.put_w(8 + 3 * k, c)
            self.put_w(10 + 3 * k, n_ij + (HT[i] - HT[j]) * (bi0 + bj0))
        def prep_u(self, t0, t1):
            R = self.R; n = R // 16
            stamps = sc.gate(t0, t1, 8 * n)
            a = lambda i, k: self.quarter(lambda r: self.w[self.kind, k, r, :], i)
            for i in range(4):
                if i % 2 == 0: tk = stamps(n)
                a1 = sc.hold(tk, a(i, 1))
                self.ubuf[self.urows(4 + i), al] = a1
                self.ubuf[self.urows(i), al] = a(i, 0) + HT[i] * a1
            for k, (i, j) in enumerate(HP):
                d1 = a(i, 1) - a(j, 1)
                n_ij = self.times(stamps(n), 1.0 / (HT[j] - HT[i]), (a(i, 0) - a(j, 0)) + HT[j] * d1)
                self.ubuf[self.urows(9 + 3 * k), al] = n_ij
                self.ubuf[self.urows(8 + 3 * k), al] = a(i, 1) - n_ij
                self.ubuf[self.urows(10 + 3 * k), al] = n_ij - d1
        def wgrad(self, lead):
            R = self.R
            def L(r, lhs):
                x = nt(lhs, jnp.concatenate([self.buf[sl(self.wid(r, q), self.wid(r, q) + 1), al] for q in range(4)], axis=1))
                filler()
                return x
            def hz(k): return s.hz[slice((self.src * 14 + k) * MQ, (self.src * 14 + k) * MQ + R), sl(0, 4)]
            def zz(i, j): return jnp.concatenate([self.quarter(lambda r: self.z[r, sl(4 * q + j, 4 * q + j + 1)], i) for q in range(4)], axis=1)
            cur = {}
            left = {(k, i): 4 + k * (3 - i) for i in range(4) for k in range(2)}
            def upd(key, x, sg=1):
                ix = self.tmp(4 * key[0] + key[1])
                if key in cur: x = s.sT[ix, :] + x if sg > 0 else s.sT[ix, :] - x
                left[key] -= 1
                cur[key] = x
                if left[key]: s.sT[ix, :] = x
            t0 = sc.now()
            for j in range(4): upd((0, j), L(j, hz(j)))
            for i in range(4): upd((1, i), L(4 + i, hz(4 + i)) + HT[i] * s.sT[self.tmp(i), :])
            stamps = sc.gate(t0 - lead, t0 + 23 * R - cfg.get("jx", 259), 6 * NGP)
            for k, (i, j) in enumerate(HP):
                self.prep_pair(k, stamps)
                c = L(8 + 3 * k, hz(8 + k))
                upd((1, i), c)
                m = L(9 + 3 * k, zz(i, j)) - c
                x = L(10 + 3 * k, zz(j, i))
                d0 = (m + x) * (1.0 / (HT[j] - HT[i]))
                d1 = HT[j] * d0 - x
                upd((0, i), d0); upd((0, j), d0, -1); upd((1, i), d1); upd((1, j), d1, -1)
                for p_ in (i, j):
                    if left[0, p_] == 0: self.emit(p_, cur[0, p_], cur[1, p_])
        def emit(self, i, d0, d1):
            if self.wix != 3: w_ = up((pltpu.bitcast(rb(d0), u32) >> 16) | pltpu.bitcast(rb(d1), u32))
            for k, (o, n) in enumerate(self.parts(i)):
                if self.wix == 3:
                    s.woo[0, o:o + n, :] = d0[k * T:k * T + n].astype(bf16)
                    s.woo[1, o:o + n, :] = d1[k * T:k * T + n].astype(bf16)
                else:
                    b0 = WOFF[self.wix] + o // 4
                    s.wout[b0:b0 + n // 4] = w_[2 * k * T:2 * (k * T + n)].reshape(n // 4, 8, D)
        def back(self):
            R = self.R
            def N(r, q): return nn(self.ubuf[self.urows(r), al], self.buf[sl(self.wid(r, q), self.wid(r, q) + 1), al])
            def cols(q, j): return sl(4 * q + j, 4 * q + j + 1)
            if self.side:
                def X(q, i): return self.tmp(12 + 10 * (q & 1) + i)
                def Y(q, j): return self.tmp(16 + 10 * (q & 1) + j)
                def put(q, i, j, x):
                    old = self.quarter(lambda r: s.acc[self.kind, r, cols(q, j)], i)
                    if self.kind == 1 and not cfg.get("init1", 1): old = jnp.where(first, 0.0, old)
                    x = old + x
                    for k, (o, n) in enumerate(self.parts(i)):
                        s.acc[self.kind, o:o + n, cols(q, j)] = x[k * T:k * T + n]
                        if self.kind == 0: s.st_x[4 * q + j, o:o + n, :] = x[k * T:k * T + n].astype(bf16)
                def xs(q, i): s.sT[X(q, i), :] = N(4 + i, q)
                def ys(q, j):
                    y = N(j, q)
                    s.sT[Y(q, j), :] = y
                    put(q, j, j, s.sT[X(q, j), :] + y)
                def off(q, i, j, c, r): put(q, i, j, ((s.sT[Y(q, j), :] - s.sT[X(q, i), :]) + c) + N(r, q))
            else:
                def get(q, i, j): return s.dcT[sl(i, i + 1), cols(q, j)]
                def off(q, i, j, c, r):
                    old = get(q, i, j)
                    if self.kind == 0: old = jnp.where(first, 0.0, old)
                    x = (old if c is None else old + c) + N(r, q)
                    s.dcT[sl(i, i + 1), cols(q, j)] = x
                    if self.kind == 1 and i != j:
                        x = x + get(q, j, j) if i == 4 else x + (get(q, 4, j) - get(q, i, i))
                        s.st_c[j if i == 4 else i, cols(q, j), :] = x.T.astype(bf16)
                def xs(q, i): off(q, i, i, None, 4 + i)
                def ys(q, j): off(q, 4, j, None, j)
            for q0 in (0, 2):
                for q in (q0, q0 + 1):
                    for i in range(4): xs(q, i)
                    filler()
                    for j in range(4): ys(q, j)
                    filler()
                jobs = [(q, k) for q in (q0, q0 + 1) for k in range(6)]
                for g0 in range(0, 12, 4):
                    qe, ke = jobs[g0 + 3]; ie, je = HP[ke]
                    held = self.tmp(20 + (g0 // 4) % 2)
                    for n in range(3):
                        q, k = jobs[g0 + n]; i, j = HP[k]
                        c = N(8 + 3 * k, q)
                        off(q, i, j, c, 9 + 3 * k)
                        off(q, j, i, c, 10 + 3 * k)
                        if n == 0: s.sT[held, :] = N(8 + 3 * ke, qe)
                        elif n == 1: off(qe, ie, je, s.sT[held, :], 9 + 3 * ke)
                        else: off(qe, je, ie, s.sT[held, :], 10 + 3 * ke)
                        filler()
    NGP = cfg.get("NGP", 32)

    mv = {}
    valid = (h >> 1) < NFC
    def hi(w): return [s.mi[w * FT + t, DC:, :] for t in range(FT)]
    def f1(w, t):
        lhs = (s.xsel, s.xsel, s.dy)[w]
        if t < FT: mv[w, t] = nn(lhs[:, :DC], s.mi[w * FT + t, :DC, :])
        else:
            x = nn(lhs[:, DC:], jnp.concatenate(hi(w), axis=1))
            mv[w, 0] = mv[w, 0] - nn(s.zero[:, :M - DC], hi(w)[0])
            mv[w] = rb(jnp.concatenate([mv[w, q] for q in range(FT)], axis=1) + x)
    def act():
        a, u, dh = mv[0], mv[1], mv[2]
        sg = sigmoid_b(a)
        g_ = rb(a * sg)
        dg = rb(dh * u)
        mv["r", 0] = rb(rb(dg * sg) + rb(rb(a * dg) * rb(sg * (1.0 - sg))))
        mv["r", 1] = rb(dh * g_)
        mv["r", 2] = rb(g_ * u)
        for w in range(3):
            for t in range(FT): s.mr[(w * FT + t) * C:(w * FT + t + 1) * C, :] = mv["r", w][:C, sl(t, t + 1)]
    def f2(w, t):
        acc = (s.dxsel, s.dxsel, s.y)[w]
        lhs = jnp.where(valid, mv["r", w], 0.0).astype(bf16)
        if t < FT: acc[:, :DC] += nt(lhs[:, sl(t, t + 1)], s.mi[w * FT + t, :DC, :])
        else: acc[:, DC:] += nt(jnp.concatenate([lhs, s.zero[...]], axis=1),
                                jnp.concatenate(hi(w) + hi(w)[:1], axis=1))
    def stamp(t): return sc.gate(t, t, 1)(1)
    ph = [Phase(0, 0), Phase(1, 0), Phase(0, 1), Phase(1, 1)]
    tw, tb = [], []
    ph[0].prep_diag()
    for n in range(4):
        tw.append(sc.now())
        if (n, cfg.get("fp", 0)) in ((2, 1), (3, 2)): fill.extend((lambda w=w, t=t: f2(w, t)) for w in range(3) for t in range(FT + 1))
        ph[n].wgrad(-cfg.get("j0", 0) if n == 0 else cfg.get("lead", 0))
        tb.append(sc.now())
        if n == 0: ph[0].prep_u(tw[0] + cfg.get("u0s", 911), tb[0] - cfg.get("u0t", 200))
        if n == 2:
            done("moe"); done("dc"); done(2, stamp(tw[2] + 400))
        if n == 3:
            done("out"); done("wo"); done(1, stamp(tw[3] + 400))
        if n == 0: fill.extend((lambda w=w, t=t: f1(w, t)) for w in range(3) for t in range(FT + 1))
        if n == 1 and not cfg.get("fp", 0): fill.extend((lambda w=w, t=t: f2(w, t)) for w in range(3) for t in range(FT + 1))
        ph[n].back()
        assert not fill
        if n == 0: act()
        if n == 3: done(0, stamp(tb[3] + 400))
        if n < 3:
            mid = tb[n] + (sc.now() - cfg.get("lead", 0) - tb[n]) * cfg.get("mid", 70) // 100
            ph[n + 1].prep_u(tb[n] + cfg.get("us", 7), mid)
            ph[n + 1].prep_diag(mid, sc.now() - cfg.get("dt", 200) - cfg.get("lead", 0))


_impl = make(dict(nobc=1, init1=0))


@jax.jit
def pallas_parallel_sum__compressed_kv_cla__moe_arch_mod__prompt_kernel(
        A_x, A_c_kv, A_w_q, A_w_uk, A_w_uv, A_w_o, B_x, B_w_r, B_w_gate, B_w_up, B_w_down, grad_out):
    return _impl(A_x, A_c_kv, A_w_q, A_w_uk, A_w_uv, A_w_o, B_x, B_w_r, B_w_gate, B_w_up, B_w_down, grad_out)
```
